```python
import jax
import jax.numpy as jnp

def _softmax(x, axis=-1):
    return jax.nn.softmax(x, axis=axis)

def _gelu(x):
    return jax.nn.gelu(x, approximate=True)

def _silu(x):
    return jax.nn.silu(x)

def _sigmoid(x):
    return jax.nn.sigmoid(x)

def _layernorm(x, axis=-1, eps=1e-05):
    m = jnp.mean(x, axis=axis, keepdims=True)
    v = jnp.var(x, axis=axis, keepdims=True)
    return (x - m) / jnp.sqrt(v + eps)

def _scatter_add(tgt, idx, src, axis=0):
    return tgt.at[idx].add(src)

def _segment_sum(src, seg, n):
    return jax.ops.segment_sum(src, seg, n)

class _Rng:

    def __init__(self, key):
        self._k = key

    def _next(self):
        self._k, sub = jax.random.split(self._k)
        return sub

    def normal(self, shape):
        return jax.random.normal(self._next(), shape, dtype=jnp.bfloat16)

    def randint(self, lo, hi, shape):
        return jax.random.randint(self._next(), shape, lo, hi, dtype=jnp.int32)

    def uniform(self, shape, lo=0.0, hi=1.0):
        return jax.random.uniform(self._next(), shape, jnp.bfloat16, lo, hi)

    def permutation(self, n):
        return jax.random.permutation(self._next(), n)
kernel_name = 'adaLN_cond__sliding_local_dilated__glu_gated_swiglu__prompt'

def setup_inputs():
    _rng = _Rng(jax.random.key(int.from_bytes(__import__("os").urandom(4), "little")))
    _w = lambda a: (lambda t: t.astype(jnp.bfloat16) if jnp.issubdtype(t.dtype, jnp.floating) else t)(jnp.asarray(a))

    def _A_setup():
        B, S, D = (1, 2048, 1024)
        return {'x': _w((lambda *s: _rng.normal(s) * 0.05)(B, S, D)), 'wqkv': _w((lambda *s: _rng.normal(s) * 0.05)(D, 3 * D)), 'wo': _w((lambda *s: _rng.normal(s) * 0.05)(D, D))}
    _A_in = _A_setup()

    def _B_setup():
        B, S, D, F = (1, 2048, 1024, 3584)
        return {'x': _w((lambda *s: _rng.normal(s) * 0.05)(B, S, D)), 'w1': _w((lambda *s: _rng.normal(s) * 0.05)(D, F) * (2.0 / D) ** 0.5), 'w3': _w((lambda *s: _rng.normal(s) * 0.05)(D, F) * (2.0 / D) ** 0.5), 'w2': _w((lambda *s: _rng.normal(s) * 0.05)(F, D) * (2.0 / F) ** 0.5)}
    _B_in = _B_setup()
    return {'A_x': _A_in['x'], 'A_wqkv': _A_in['wqkv'], 'A_wo': _A_in['wo'], 'B_x': _B_in['x'], 'B_w1': _B_in['w1'], 'B_w3': _B_in['w3'], 'B_w2': _B_in['w2'], 'c': _w((lambda *s: _rng.normal(s) * 0.05)(1, 1024)), 'w_mod': _w((lambda *s: _rng.normal(s) * 0.05)(1024, 6 * 1024) * 1024 ** (-0.5))}

def reference(A_x, A_wqkv, A_wo, B_x, B_w1, B_w3, B_w2, c, w_mod):

    def _A_ref(x, wqkv, wo):
        B, S, D = x.shape
        H = 32
        Dh = D // H
        W, dil = (8, 2)
        qkv = (lambda x, *d: x.transpose(*d))((x @ wqkv).reshape(B, S, 3, H, Dh), 2, 0, 3, 1, 4)
        q, k, v = (qkv[0], qkv[1], qkv[2])
        scale = Dh ** (-0.5)
        pos = jnp.arange(S)
        off = jnp.arange(W) * dil
        idx = pos[:, None] - off[None, :]
        mask = idx >= 0
        idx_c = jnp.where(mask, idx, 0).reshape(-1)
        kg = k[:, :, idx_c, :].reshape(B, H, S, W, Dh)
        vg = v[:, :, idx_c, :].reshape(B, H, S, W, Dh)
        logits = jnp.einsum('bhsd,bhswd->bhsw', q, kg) * scale
        logits = jnp.where(mask[None, None, :, :], logits, -1000000000.0)
        attn = _softmax(logits, axis=-1)
        o = jnp.einsum('bhsw,bhswd->bhsd', attn, vg)
        return (lambda x, *d: x.transpose(*d))(o, 0, 2, 1, 3).reshape(B, S, D) @ wo

    def _B_ref(x, w1, w3, w2):
        gate = jnp.einsum('bsd,df->bsf', x, w1)
        up = jnp.einsum('bsd,df->bsf', x, w3)
        h = _silu(gate) * up
        out = jnp.einsum('bsf,fd->bsd', h, w2)
        return out
    x = A_x
    mod = (_silu(c) @ w_mod).reshape(c.shape[0], 6, 1, -1)
    sa, ca, ga, sb, cb, gb = (mod[:, 0].copy(), mod[:, 1].copy(), mod[:, 2].copy(), mod[:, 3].copy(), mod[:, 4].copy(), mod[:, 5].copy())
    h = _layernorm(x, axis=-1) * (1 + ca) + sa
    x = x + ga * _A_ref(h, A_wqkv, A_wo)
    h = _layernorm(x, axis=-1) * (1 + cb) + sb
    x = x + gb * _B_ref(h, B_w1, B_w3, B_w2)
    return x
```

```python
import functools
import math
import jax
import jax.numpy as jnp
import numpy as np
from jax import lax
from jax.experimental import pallas as pl
from jax.experimental.pallas import tpu as pltpu

S, D, F, H, DH, W, DIL = 2048, 1024, 3584, 32, 32, 8, 2
EPS = 1e-5
T = 256
FC = 512
HALO = 16
NT = D // 128
RC = 16
ORDER = 2
TAILFFN = True
FLAGS = {"XLA_TPU_EVENLY_DISTRIBUTE_CRITICAL_NODES": True}
f32, bf16, u32 = jnp.float32, jnp.bfloat16, jnp.uint32
NTDIMS = (((1,), (1,)), ((), ()))


def _ln_mod(x, scale1, shift):
    m = jnp.mean(x, axis=-1, keepdims=True)
    xc = x - m
    v = jnp.mean(xc * xc, axis=-1, keepdims=True)
    return xc * lax.rsqrt(v + EPS) * scale1 + shift


def _group_allreduce(s):
    lane = lax.broadcasted_iota(jnp.int32, s.shape, 1)
    s = s + jnp.where((lane & 1) == 0, pltpu.roll(s, 127, 1), pltpu.roll(s, 1, 1))
    s = s + jnp.where((lane & 2) == 0, pltpu.roll(s, 126, 1), pltpu.roll(s, 2, 1))
    return s


def _rowperm(X):
    C = X[0].shape[1]
    U = [pltpu.bitcast(x, u32) for x in X]
    out = [[None] * 8 for _ in range(8)]
    sub = lax.broadcasted_iota(jnp.int32, (8, C), 0)
    m4 = (sub & 4) == 0
    m2 = (sub & 2) == 0
    for a in range(4):
        for j2 in range(2):
            Z = [U[b][(a * 2 + j2) * 8:(a * 2 + j2 + 1) * 8] for b in range(8)]
            for bit, s, m in ((2, 4, m4), (1, 2, m2)):
                for b in range(8):
                    if b & bit == 0:
                        A, B = Z[b], Z[b | bit]
                        Z[b] = jnp.where(m, A, pltpu.roll(B, s, 0))
                        Z[b | bit] = jnp.where(m, pltpu.roll(A, 8 - s, 0), B)
            for b in range(8):
                b2, j1, j0 = b >> 2, (b >> 1) & 1, b & 1
                out[j2 * 4 + j1 * 2 + j0][a * 2 + b2] = Z[b]
    return [pltpu.bitcast(jnp.concatenate(o, 0), bf16) for o in out]


def _kernel(x_hbm, wqkv_hbm, wo_hbm, w1_hbm, w3_hbm, w2_hbm, c_hbm, wmod_hbm, o_hbm,
            xv, wraw, wt, wo_raw, wo, w1, w3, w2, cv, wmod, mod,
            hA, hB, kA, kB, vA, vB, qA, qB, oA, oB, x1buf, h2buf, outv, sems, osems):
    NB = S // T
    sem_i = [0]

    def cp(src, dst):
        i = sem_i[0]; sem_i[0] += 1
        return pltpu.make_async_copy(src, dst, sems.at[i])

    def cols(ref, a, n):
        return ref.at[:, pl.ds(a, n)]

    def rows(ref, a, n):
        return ref.at[pl.ds(a, n), :]

    plan = []
    def add(name, src, dst):
        plan.append((name, cp(src, dst)))
    add("c", c_hbm, cv)
    add("x0", rows(x_hbm, 0, 2 * T), rows(xv, 0, 2 * T))
    for p in range(8):
        add(f"ma{p}", cols(wmod_hbm, p * 256, 256), cols(wmod, p * 256, 256))
    for kq in range(8):
        add(f"wq{kq}", rows(wqkv_hbm, kq * 128, 128), rows(wraw, kq * 128, 128))
    add("wo", wo_hbm, wo_raw)
    add("mga", cols(wmod_hbm, 2048, 1024), cols(wmod, 2048, 1024))
    add("x1", rows(x_hbm, 2 * T, S - 2 * T), rows(xv, 2 * T, S - 2 * T))
    add("mb", cols(wmod_hbm, 3072, 3072), cols(wmod, 3072, 3072))
    add("w1", w1_hbm, w1)
    add("w3", w3_hbm, w3)
    add("w2", w2_hbm, w2)
    names = [n for n, _ in plan]
    state = {"issued": 0, "waited": 0}
    INFLIGHT = 3

    def pump():
        while state["issued"] < len(plan) and state["issued"] < state["waited"] + INFLIGHT:
            plan[state["issued"]][1].start(); state["issued"] += 1

    def need(name):
        idx = names.index(name)
        while state["waited"] <= idx:
            pump()
            plan[state["waited"]][1].wait(); state["waited"] += 1
        pump()

    pump()
    need("c")
    cc = cv[...].astype(f32)
    sc = jnp.broadcast_to(cc * jax.nn.sigmoid(cc), (8, D)).astype(bf16)
    for j in range(NT):
        kA[j, 0:HALO, :] = jnp.zeros((HALO, 128), f32)
        vA[j, 0:HALO, :] = jnp.zeros((HALO, 128), f32)
    for p in range(8):
        need(f"ma{p}")
        mod[:, p * 256:(p + 1) * 256] = jnp.dot(sc, wmod[:, p * 256:(p + 1) * 256], preferred_element_type=f32)

    def row0(i):
        return i * T if isinstance(i, int) else pl.multiple_of(i * T, T)

    def ln1(i, h_ref):
        x = xv[pl.ds(row0(i), T), :].astype(f32)
        h_ref[...] = _ln_mod(x, 1.0 + mod[0:1, 1024:2048], mod[0:1, 0:1024]).astype(bf16)

    ln1(0, hA)
    for kq in range(8):
        need(f"wq{kq}")
        for m in range(3):
            X = [wraw[kq * 128:(kq + 1) * 128, m * D + b * 128:m * D + (b + 1) * 128].T for b in range(NT)]
            Y = _rowperm(X)
            for j in range(NT):
                wt[m * D + j * 128:m * D + (j + 1) * 128, kq * 128:(kq + 1) * 128] = Y[j]
    qscale = DH ** -0.5 * math.log2(math.e)

    def proj_tiles(h, c0, dst, r0):
        y = lax.dot_general(h, wt[c0:c0 + D, :], NTDIMS, preferred_element_type=f32)
        for j in range(NT):
            dst[j, r0:r0 + T, :] = y[:, j * 128:(j + 1) * 128]

    def attn1(i, qbuf, k_ref, c):
        rs = slice(c * RC, (c + 1) * RC)
        qt = [qbuf[j, rs, :] for j in range(NT)]
        ls = []
        for w in range(W):
            o = HALO - DIL * w + c * RC
            s = None
            for j in range(NT):
                p = qt[j] * k_ref[j, o:o + RC, :]
                s = p if s is None else s + p
            s = _group_allreduce(s) * qscale
            if w > 0 and c * RC < DIL * w:
                row = row0(i) + c * RC + lax.broadcasted_iota(jnp.int32, (RC, 128), 0)
                s = jnp.where(row >= DIL * w, s, -1.5e9)
            ls.append(s)
        return ls

    def attn2(ls, v_ref, obuf, c):
        rs = slice(c * RC, (c + 1) * RC)
        m = functools.reduce(jnp.maximum, ls)
        es = [jnp.exp2(l - m) for l in ls]
        r = 1.0 / functools.reduce(jnp.add, es)
        ps = [e * r for e in es]
        for j in range(NT):
            acc = None
            for w in range(W):
                o = HALO - DIL * w + c * RC
                p = ps[w] * v_ref[j, o:o + RC, :]
                acc = p if acc is None else acc + p
            obuf[rs, j * 128:(j + 1) * 128] = acc.astype(bf16)

    def attn(i, qbuf, k_ref, v_ref, obuf):
        for c in range(T // RC):
            attn2(attn1(i, qbuf, k_ref, c), v_ref, obuf, c)

    def ln2(i):
        x1 = x1buf[pl.ds(row0(i), T), :]
        h2buf[pl.ds(row0(i), T), :] = _ln_mod(x1, 1.0 + mod[0:1, 4096:5120], mod[0:1, 3072:4096]).astype(bf16)

    Hs = (hA, hB); Ks = (kA, kB); Vs = (vA, vB); Qs = (qA, qB); Os = (oA, oB)

    def qkv(i):
        p = i % 2
        h = Hs[p][...]
        if i > 0:
            for j in range(NT):
                Ks[p][j, 0:HALO, :] = Ks[1 - p][j, T:T + HALO, :]
                Vs[p][j, 0:HALO, :] = Vs[1 - p][j, T:T + HALO, :]
        proj_tiles(h, 0, Qs[p], 0)
        proj_tiles(h, D, Ks[p], HALO)
        proj_tiles(h, 2 * D, Vs[p], HALO)

    def wo_x1(i):
        a = jnp.dot(Os[i % 2][...], wo[...], preferred_element_type=f32)
        x1 = xv[pl.ds(row0(i), T), :].astype(f32) + mod[0:1, 2048:3072] * a
        x1buf[pl.ds(row0(i), T), :] = x1

    def ffn(i, has_next, extra=None):
        r0 = row0(i)
        h = h2buf[pl.ds(r0, T), :]
        if has_next:
            ln2(i + 1)
        acc = None
        for f in range(F // FC):
            fs = slice(f * FC, (f + 1) * FC)
            g = jnp.dot(h, w1[:, fs], preferred_element_type=f32)
            u = jnp.dot(h, w3[:, fs], preferred_element_type=f32)
            a = (g * jax.nn.sigmoid(g) * u).astype(bf16)
            d = jnp.dot(a, w2[fs, :], preferred_element_type=f32)
            acc = d if acc is None else acc + d
            if extra is not None:
                extra(f)
        outv[pl.ds(r0, T), :] = (x1buf[pl.ds(r0, T), :] + mod[0:1, 5120:6144] * acc).astype(bf16)
        pltpu.make_async_copy(outv.at[pl.ds(r0, T), :], o_hbm.at[pl.ds(r0, T), :], osems.at[i]).start()

    for i in range(-1, NB + 1):
        def st_ln1():
            if 1 <= i + 2 < NB: ln1(i + 2, Hs[(i + 2) % 2])
        def st_qkv():
            if 0 <= i + 1 < NB: qkv(i + 1)
        def st_att():
            if 0 <= i < NB: attn(i, Qs[i % 2], Ks[i % 2], Vs[i % 2], Os[i % 2])
        def st_wo():
            if 0 <= i - 1 < NB: wo_x1(i - 1)
        if i == 0:
            need("wo")
            for cb in range(NT):
                X = [wo_raw[b * 128:(b + 1) * 128, cb * 128:(cb + 1) * 128] for b in range(NT)]
                Y = _rowperm(X)
                for j in range(NT):
                    wo[j * 128:(j + 1) * 128, cb * 128:(cb + 1) * 128] = Y[j]
            need("mga")
            mod[:, 2048:3072] = jnp.dot(sc, wmod[:, 2048:3072], preferred_element_type=f32)
            need("x1")
        if i == 1:
            need("mb")
            mod[:, 3072:6144] = jnp.dot(sc, wmod[:, 3072:6144], preferred_element_type=f32)
        if i == NB - 1:
            need("w2")
        if TAILFFN and i == NB - 1:
            st_wo(); ffn(0, True); st_att()
        else:
            st_wo(); st_qkv(); st_att(); st_ln1()
        if i == 2:
            ln2(0)

    first = 1 if TAILFFN else 0
    lax.fori_loop(first, NB - 1, lambda i, c: (ffn(i, True), 0)[1], 0)
    ffn(NB - 1, False)
    for i in range(NB):
        pltpu.make_async_copy(outv.at[pl.ds(i * T, T), :], o_hbm.at[pl.ds(i * T, T), :], osems.at[i]).wait()


def pallas_adaLN_cond__sliding_local_dilated__glu_gated_swiglu__prompt_kernel(
        A_x, A_wqkv, A_wo, B_x, B_w1, B_w3, B_w2, c, w_mod):
    NB = S // T
    anyspec = pl.BlockSpec(memory_space=pl.ANY)
    kv_shape = pltpu.VMEM((NT, T + HALO, 128), f32)
    out = pl.pallas_call(
        _kernel,
        out_shape=jax.ShapeDtypeStruct((S, D), bf16),
        in_specs=[anyspec] * 8,
        out_specs=anyspec,
        scratch_shapes=[
            pltpu.VMEM((S, D), bf16),
            pltpu.VMEM((D, 3 * D), bf16),
            pltpu.VMEM((3 * D, D), bf16),
            pltpu.VMEM((D, D), bf16),
            pltpu.VMEM((D, D), bf16),
            pltpu.VMEM((D, F), bf16),
            pltpu.VMEM((D, F), bf16),
            pltpu.VMEM((F, D), bf16),
            pltpu.VMEM((1, D), bf16),
            pltpu.VMEM((D, 6 * D), bf16),
            pltpu.VMEM((8, 6 * D), f32),
            pltpu.VMEM((T, D), bf16), pltpu.VMEM((T, D), bf16),
            kv_shape, kv_shape, kv_shape, kv_shape,
            pltpu.VMEM((NT, T, 128), f32), pltpu.VMEM((NT, T, 128), f32),
            pltpu.VMEM((T, D), bf16), pltpu.VMEM((T, D), bf16),
            pltpu.VMEM((S, D), f32),
            pltpu.VMEM((S, D), bf16),
            pltpu.VMEM((S, D), bf16),
            pltpu.SemaphoreType.DMA((40,)),
            pltpu.SemaphoreType.DMA((NB,)),
        ],
        compiler_params=pltpu.CompilerParams(vmem_limit_bytes=120 * 1024 * 1024, flags=FLAGS),
    )(A_x.reshape(S, D), A_wqkv, A_wo, B_w1, B_w3, B_w2, c, w_mod)
    return out.reshape(1, S, D)
```

```python
import functools
import math
import jax
import jax.numpy as jnp
import numpy as np
from jax import lax
from jax.experimental import pallas as pl
from jax.experimental.pallas import tpu as pltpu

S, D, F, H, DH, W, DIL = 2048, 1024, 3584, 32, 32, 8, 2
EPS = 1e-5
T = 256
FC = 512
HALO = 16
NT = D // 128
RC = 8
KCH = (128, 128, 256, 256, 256)
INFLIGHT = 6
ASPAN = 0.875
LSPAN = 0.75
LNP = 8
LNOFF = 1
TAILSPLIT = 3
AORDER = 0
EVEN = True
f32, bf16, u32 = jnp.float32, jnp.bfloat16, jnp.uint32


def _group_allreduce(s):
    lane = lax.broadcasted_iota(jnp.int32, s.shape, 1)
    s = s + jnp.where((lane & 1) == 0, pltpu.roll(s, 127, 1), pltpu.roll(s, 1, 1))
    s = s + jnp.where((lane & 2) == 0, pltpu.roll(s, 126, 1), pltpu.roll(s, 2, 1))
    return s


def _butterfly(X):
    X = list(X)
    lane = lax.broadcasted_iota(jnp.int32, X[0].shape, 1)
    for b, s in ((1, 4), (2, 8), (4, 16)):
        m = (lane & s) == 0
        for i in range(NT):
            if i & b == 0:
                A, B = X[i], X[i | b]
                X[i] = jnp.where(m, A, pltpu.roll(B, s, 1))
                X[i | b] = jnp.where(m, pltpu.roll(A, 128 - s, 1), B)
    return X


def _rowperm(X):
    C = X[0].shape[1]
    U = [pltpu.bitcast(x, u32) for x in X]
    out = [[None] * 8 for _ in range(8)]
    sub = lax.broadcasted_iota(jnp.int32, (8, C), 0)
    m4 = (sub & 4) == 0
    m2 = (sub & 2) == 0
    for a in range(4):
        for j2 in range(2):
            Z = [U[b][(a * 2 + j2) * 8:(a * 2 + j2 + 1) * 8] for b in range(8)]
            for bit, s, m in ((2, 4, m4), (1, 2, m2)):
                for b in range(8):
                    if b & bit == 0:
                        A, B = Z[b], Z[b | bit]
                        Z[b] = jnp.where(m, A, pltpu.roll(B, s, 0))
                        Z[b | bit] = jnp.where(m, pltpu.roll(A, 8 - s, 0), B)
            for b in range(8):
                b2, j1, j0 = b >> 2, (b >> 1) & 1, b & 1
                out[j2 * 4 + j1 * 2 + j0][a * 2 + b2] = Z[b]
    return [pltpu.bitcast(jnp.concatenate(o, 0), bf16) for o in out]


def _kernel(x_hbm, wqkv_hbm, wo_hbm, w1_hbm, w3_hbm, w2_hbm, c_hbm, wmod_hbm, o_hbm,
            xv, wqkv, xh, wo_raw, wo, w1, w3, w2, cv, wmod, mod,
            hA, hB, hS, kA, kB, kC, vA, vB, vC, qA, qB, qC, oA, oB, x1buf, h2buf, outv, sems, osems):
    NB = S // T
    sem_i = [0]

    def cp(src, dst):
        i = sem_i[0]; sem_i[0] += 1
        return pltpu.make_async_copy(src, dst, sems.at[i])

    def cols(ref, a, n):
        return ref.at[:, pl.ds(a, n)]

    def rows(ref, a, n):
        return ref.at[pl.ds(a, n), :]

    plan = []
    def add(name, src, dst):
        plan.append((name, cp(src, dst)))
    kofs = [sum(KCH[:i]) for i in range(len(KCH))]
    assert sum(KCH) == D
    add("c", c_hbm, cv)
    add("x0", rows(x_hbm, 0, 2 * T), rows(xv, 0, 2 * T))
    for q, (k0, kn) in enumerate(zip(kofs, KCH)):
        add(f"ms{q}", cols(wmod_hbm, k0, kn), cols(wmod, k0, kn))
        add(f"mc{q}", cols(wmod_hbm, D + k0, kn), cols(wmod, D + k0, kn))
        add(f"wq{q}", rows(wqkv_hbm, k0, kn), rows(wqkv, k0, kn))
    add("x2", rows(x_hbm, 2 * T, 2 * T), rows(xv, 2 * T, 2 * T))
    add("wo", wo_hbm, wo_raw)
    add("mga", cols(wmod_hbm, 2048, 1024), cols(wmod, 2048, 1024))
    add("x1", rows(x_hbm, 4 * T, S - 4 * T), rows(xv, 4 * T, S - 4 * T))
    add("mb", cols(wmod_hbm, 3072, 3072), cols(wmod, 3072, 3072))
    add("w1", w1_hbm, w1)
    add("w3", w3_hbm, w3)
    add("w2", w2_hbm, w2)
    names = [n for n, _ in plan]
    state = {"issued": 0, "waited": 0}

    def pump():
        while state["issued"] < len(plan) and state["issued"] < state["waited"] + INFLIGHT:
            plan[state["issued"]][1].start(); state["issued"] += 1

    def need(name):
        idx = names.index(name)
        while state["waited"] <= idx:
            pump()
            plan[state["waited"]][1].wait(); state["waited"] += 1
        pump()

    pump()
    need("c")
    cc = cv[...].astype(f32)
    sc = jnp.broadcast_to(cc * jax.nn.sigmoid(cc), (8, D)).astype(bf16)
    pred = (pltpu.bitcast(jnp.broadcast_to(cc[:, 0:128], (8, 128)), jnp.int32) | 1) != 0

    def gate(val, y):
        if y is None:
            return val
        return jnp.where(pred, jnp.full((8, 128), val, f32), y)

    for j in range(NT):
        kA[j, 0:HALO, :] = jnp.zeros((HALO, 128), f32)
        vA[j, 0:HALO, :] = jnp.zeros((HALO, 128), f32)

    Hs = (hA, hB); Ks = (kA, kB, kC); Vs = (vA, vB, vC); Qs = (qA, qB, qC); Os = (oA, oB)
    qscale = DH ** -0.5 * math.log2(math.e)

    def ln_rows(src, dst, r_src, r_dst, rn, c_scale, c_shift, g):
        x = src[pl.ds(r_src, rn), :].astype(f32)
        sm = jnp.sum(x, axis=-1, keepdims=True)
        if g is None:
            m = sm * (1.0 / D)
        else:
            gv = gate(1.0 / D, g)
            m = sm * jnp.concatenate([gv] * (rn // 8), axis=0)[:, 0:1]
        xc = x - m
        v = jnp.mean(xc * xc, axis=-1, keepdims=True)
        hh = xc * lax.rsqrt(v + EPS) * (1.0 + mod[0:1, c_scale:c_scale + D]) + mod[0:1, c_shift:c_shift + D]
        dst[pl.ds(r_dst, rn), :] = hh.astype(bf16)

    def ln1_piece(i, q, g):
        rn = T // LNP
        ln_rows(xv, Hs[i % 2], i * T + q * rn, q * rn, rn, D, 0, g)

    def ln2_piece(i, q, g):
        rn = T // LNP
        ln_rows(x1buf, h2buf, i * T + q * rn, i * T + q * rn, rn, 4 * D, 3 * D, g)

    need("x0")
    x01 = xv[0:2 * T, :].astype(f32)
    m01 = jnp.mean(x01, axis=-1, keepdims=True)
    xc01 = x01 - m01
    xh[...] = xc01 * lax.rsqrt(jnp.mean(xc01 * xc01, axis=-1, keepdims=True) + EPS)

    def stage_a(q):
        k0, kn = kofs[q], KCH[q]
        need(f"mc{q}")
        sa = jnp.dot(sc, wmod[:, k0:k0 + kn], preferred_element_type=f32)
        ca = jnp.dot(sc, wmod[:, D + k0:D + k0 + kn], preferred_element_type=f32)
        mod[:, k0:k0 + kn] = sa
        mod[:, D + k0:D + k0 + kn] = ca
        hS[:, k0:k0 + kn] = (xh[:, k0:k0 + kn] * (1.0 + ca[0:1, :]) + sa[0:1, :]).astype(bf16)
        need(f"wq{q}")
        for m in range(3):
            X = [pltpu.bitcast(wqkv[k0:k0 + kn, m * D + j * 128:m * D + (j + 1) * 128], u32) for j in range(NT)]
            X = _butterfly(X)
            for j in range(NT):
                wqkv[k0:k0 + kn, m * D + j * 128:m * D + (j + 1) * 128] = pltpu.bitcast(X[j], bf16)

    def stage_b(q):
        k0, kn = kofs[q], KCH[q]
        for blk in range(2):
            h = hS[blk * T:(blk + 1) * T, k0:k0 + kn]
            for m, (bufs, r0) in enumerate(((Qs, 0), (Ks, HALO), (Vs, HALO))):
                y = jnp.dot(h, wqkv[k0:k0 + kn, m * D:(m + 1) * D], preferred_element_type=f32)
                dst = bufs[blk]
                for j in range(NT):
                    if q == 0:
                        dst[j, r0:r0 + T, :] = y[:, j * 128:(j + 1) * 128]
                    else:
                        dst[j, r0:r0 + T, :] = dst[j, r0:r0 + T, :] + y[:, j * 128:(j + 1) * 128]

    NQ = len(KCH)
    stage_a(0)
    for q in range(NQ):
        if q + 1 < NQ:
            if AORDER == 0:
                stage_a(q + 1); stage_b(q)
            else:
                need(f"wq{q + 1}")
                stage_b(q); stage_a(q + 1)
        else:
            need("x2")
            stage_b(q)
            for p in range(LNP):
                ln1_piece(2, p, None)
    for j in range(NT):
        Ks[1][j, 0:HALO, :] = Ks[0][j, T:T + HALO, :]
        Vs[1][j, 0:HALO, :] = Vs[0][j, T:T + HALO, :]

    def attn_chunk(i, c, g):
        qbuf, k_ref, v_ref, obuf = Qs[i % 3], Ks[i % 3], Vs[i % 3], Os[i % 2]
        rs = slice(c * RC, (c + 1) * RC)
        sg = gate(qscale, g)
        if g is not None and RC > 8:
            sg = jnp.concatenate([sg] * (RC // 8), axis=0)
        qt = [qbuf[j, rs, :] * sg for j in range(NT)]
        ls = []
        for w in range(W):
            o = HALO - DIL * w + c * RC
            s = None
            for j in range(NT):
                p = qt[j] * k_ref[j, o:o + RC, :]
                s = p if s is None else s + p
            s = _group_allreduce(s)
            if i == 0 and c * RC < DIL * w:
                row = c * RC + lax.broadcasted_iota(jnp.int32, (RC, 128), 0)
                s = jnp.where(row >= DIL * w, s, -1.5e9)
            ls.append(s)
        m = functools.reduce(jnp.maximum, ls)
        es = [jnp.exp2(l - m) for l in ls]
        r = 1.0 / functools.reduce(jnp.add, es)
        ps = [e * r for e in es]
        for j in range(NT):
            acc = None
            for w in range(W):
                o = HALO - DIL * w + c * RC
                p = ps[w] * v_ref[j, o:o + RC, :]
                acc = p if acc is None else acc + p
            obuf[rs, j * 128:(j + 1) * 128] = acc.astype(bf16)

    def qkv_items(i):
        p, pp = i % 3, (i - 1) % 3
        st = {}
        def mk(n):
            def run():
                if n == 0:
                    for j in range(NT):
                        Ks[p][j, 0:HALO, :] = Ks[pp][j, T:T + HALO, :]
                        Vs[p][j, 0:HALO, :] = Vs[pp][j, T:T + HALO, :]
                    st["h"] = Hs[i % 2][...]
                y = jnp.dot(st["h"], wqkv[:, n * 128:(n + 1) * 128], preferred_element_type=f32)
                dst, r0 = ((Qs[p], 0), (Ks[p], HALO), (Vs[p], HALO))[n // NT]
                dst[n % NT, r0:r0 + T, :] = y
                return y[T - 8:T, :]
            return run
        return [mk(n) for n in range(3 * NT)]

    def wo_items(i):
        st = {}
        def mk(n):
            def run():
                if n == 0:
                    st["o"] = Os[i % 2][...]
                cs = slice(n * 128, (n + 1) * 128)
                a = jnp.dot(st["o"], wo[:, cs], preferred_element_type=f32)
                x1buf[i * T:(i + 1) * T, cs] = xv[i * T:(i + 1) * T, cs].astype(f32) + mod[0:1, 2 * D + n * 128:2 * D + (n + 1) * 128] * a
                return a[T - 8:T, :]
            return run
        return [mk(n) for n in range(NT)]

    def ffn_items(i, r0):
        st = {"acc": None, "h": None}
        items = []
        def chunk(f):
            def run():
                if st["h"] is None:
                    st["h"] = h2buf[pl.ds(r0, T), :]
                h = st["h"]
                fs = slice(f * FC, (f + 1) * FC)
                g = jnp.dot(h, w1[:, fs], preferred_element_type=f32)
                u = jnp.dot(h, w3[:, fs], preferred_element_type=f32)
                a = (g * jax.nn.sigmoid(g) * u).astype(bf16)
                d = jnp.dot(a, w2[fs, :], preferred_element_type=f32)
                st["acc"] = d if st["acc"] is None else st["acc"] + d
                return [g[T - 8:T, 0:128], g[T - 8:T, FC - 128:FC], u[T - 8:T, 0:128], u[T - 8:T, FC - 128:FC],
                        d[T - 8:T, 0:128], d[T - 8:T, D - 128:D]]
            return run
        def fin():
            outv[pl.ds(r0, T), :] = (x1buf[pl.ds(r0, T), :] + mod[0:1, 5 * D:6 * D] * st["acc"]).astype(bf16)
            pltpu.make_async_copy(outv.at[pl.ds(r0, T), :], o_hbm.at[pl.ds(r0, T), :], osems.at[i]).start()
            return []
        return st, [chunk(f) for f in range(F // FC)] + [fin]

    def run_paced(mx, vec):
        evs_total = len(mx)
        vec = sorted(vec, key=lambda t: t[0])
        vi = 0
        for e, item in enumerate(mx):
            y = item()
            if isinstance(y, list):
                y = y[-1] if y else None
            while vi < len(vec) and vec[vi][0] * evs_total < e + 1:
                vec[vi][1](y); vi += 1
        while vi < len(vec):
            vec[vi][1](None); vi += 1

    NC = T // RC

    def att_vec(i, lo=0.0, span=ASPAN):
        return [(lo + span * c / NC, functools.partial(attn_chunk, i, c)) for c in range(NC)]

    def ln1_vec(i, lo, span):
        return [(lo + span * q / LNP, functools.partial(ln1_piece, i, q)) for q in range(LNP)]

    def ln2_vec(i, lo, span):
        return [(lo + span * q / LNP, functools.partial(ln2_piece, i, q)) for q in range(LNP)]

    tail_st, tail = ffn_items(0, 0)
    for i in range(0, NB + 1):
        if i == 0:
            need("wo")
            for cb in range(NT):
                X = [wo_raw[b * 128:(b + 1) * 128, cb * 128:(cb + 1) * 128] for b in range(NT)]
                Y = _rowperm(X)
                for j in range(NT):
                    wo[j * 128:(j + 1) * 128, cb * 128:(cb + 1) * 128] = Y[j]
            need("mga")
            mod[:, 2048:3072] = jnp.dot(sc, wmod[:, 2048:3072], preferred_element_type=f32)
            need("x1")
        if i == 1:
            need("mb")
            mod[:, 3072:6144] = jnp.dot(sc, wmod[:, 3072:6144], preferred_element_type=f32)
        if i == NB - 2:
            need("w2")
        mx, vec = [], []
        if i >= 1:
            mx += wo_items(i - 1)
        if i + 2 < NB:
            mx += qkv_items(i + 2)
        if i < NB:
            vec += att_vec(i)
        if i + 3 < NB:
            vec += ln1_vec(i + 3, LNOFF / 32, LSPAN)
        if i == 5:
            vec += ln2_vec(0, 0.1, 0.4) + ln2_vec(1, 0.5, 0.4)
        if i == NB - 2:
            mx += tail[:TAILSPLIT]
        if i == NB - 1:
            mx += tail[TAILSPLIT:]
        run_paced(mx, vec)

    def ffn(i, has_next):
        r0 = pl.multiple_of(i * T, T)
        st, items = ffn_items(i, r0)
        st["h"] = h2buf[pl.ds(r0, T), :]
        if has_next:
            ln_rows(x1buf, h2buf, r0 + T, r0 + T, T, 4 * D, 3 * D, None)
        for t in items:
            t()

    lax.fori_loop(1, NB - 1, lambda i, c: (ffn(i, True), 0)[1], 0)
    ffn(NB - 1, False)
    for i in range(NB):
        pltpu.make_async_copy(outv.at[pl.ds(i * T, T), :], o_hbm.at[pl.ds(i * T, T), :], osems.at[i]).wait()


def pallas_adaLN_cond__sliding_local_dilated__glu_gated_swiglu__prompt_kernel(
        A_x, A_wqkv, A_wo, B_x, B_w1, B_w3, B_w2, c, w_mod):
    NB = S // T
    anyspec = pl.BlockSpec(memory_space=pl.ANY)
    kv_shape = pltpu.VMEM((NT, T + HALO, 128), f32)
    flags = {"XLA_TPU_EVENLY_DISTRIBUTE_CRITICAL_NODES": True} if EVEN else {}
    out = pl.pallas_call(
        _kernel,
        out_shape=jax.ShapeDtypeStruct((S, D), bf16),
        in_specs=[anyspec] * 8,
        out_specs=anyspec,
        scratch_shapes=[
            pltpu.VMEM((S, D), bf16),
            pltpu.VMEM((D, 3 * D), bf16),
            pltpu.VMEM((2 * T, D), f32),
            pltpu.VMEM((D, D), bf16),
            pltpu.VMEM((D, D), bf16),
            pltpu.VMEM((D, F), bf16),
            pltpu.VMEM((D, F), bf16),
            pltpu.VMEM((F, D), bf16),
            pltpu.VMEM((1, D), bf16),
            pltpu.VMEM((D, 6 * D), bf16),
            pltpu.VMEM((8, 6 * D), f32),
            pltpu.VMEM((T, D), bf16), pltpu.VMEM((T, D), bf16), pltpu.VMEM((2 * T, D), bf16),
            kv_shape, kv_shape, kv_shape, kv_shape, kv_shape, kv_shape,
            pltpu.VMEM((NT, T, 128), f32), pltpu.VMEM((NT, T, 128), f32), pltpu.VMEM((NT, T, 128), f32),
            pltpu.VMEM((T, D), bf16), pltpu.VMEM((T, D), bf16),
            pltpu.VMEM((S, D), f32),
            pltpu.VMEM((S, D), bf16),
            pltpu.VMEM((S, D), bf16),
            pltpu.SemaphoreType.DMA((40,)),
            pltpu.SemaphoreType.DMA((NB,)),
        ],
        compiler_params=pltpu.CompilerParams(vmem_limit_bytes=120 * 1024 * 1024, flags=flags),
    )(A_x.reshape(S, D), A_wqkv, A_wo, B_w1, B_w3, B_w2, c, w_mod)
    return out.reshape(1, S, D)
```

```python
import contextlib
import functools
import math
import jax
import jax.numpy as jnp
import numpy as np
from jax import lax
from jax.experimental import pallas as pl
from jax.experimental.pallas import tpu as pltpu

S, D, F, H, DH, W, DIL = 2048, 1024, 3584, 32, 32, 8, 2
EPS = 1e-5
T = 256
FC = 512
HALO = 16
NT = D // 128
RC = 8
KCH = (128,) * 8
PRG = 64
PRG0 = 128
OFF_W = 3
OFF_C = 2
OFF_H = 2
OFF_P = (3, 1, -1)
OFFGROW = 1
OFFMAX = 6
ONEDOT = False
VMOD = True
VMODB = False
HALFW = True
LN0P = 4
ASPAN = 0.875
LSPAN = 0.75
LNP = 8
LNOFF = 1
TAILSPLIT = 3
TSPAN = 0.9
MODB_AT = 3
WOPREP = 0.3
EVEN = True
SCOPES = False
XSPLIT = True
GATEP = False
f32, bf16, u32 = jnp.float32, jnp.bfloat16, jnp.uint32


def scope(name):
    return jax.named_scope(name) if SCOPES else contextlib.nullcontext()


def _group_allreduce(s):
    lane = lax.broadcasted_iota(jnp.int32, s.shape, 1)
    s = s + jnp.where((lane & 1) == 0, pltpu.roll(s, 127, 1), pltpu.roll(s, 1, 1))
    s = s + jnp.where((lane & 2) == 0, pltpu.roll(s, 126, 1), pltpu.roll(s, 2, 1))
    return s


def _butterfly(X, lane=None):
    X = list(X)
    if lane is None:
        lane = lax.broadcasted_iota(jnp.int32, X[0].shape, 1)
    for b, s in ((1, 4), (2, 8), (4, 16)):
        m = (lane & s) == 0
        for i in range(NT):
            if i & b == 0:
                A, B = X[i], X[i | b]
                X[i] = jnp.where(m, A, pltpu.roll(B, s, 1))
                X[i | b] = jnp.where(m, pltpu.roll(A, 128 - s, 1), B)
    return X


def _rowperm(X):
    C = X[0].shape[1]
    U = [pltpu.bitcast(x, u32) for x in X]
    out = [[None] * 8 for _ in range(8)]
    sub = lax.broadcasted_iota(jnp.int32, (8, C), 0)
    m4 = (sub & 4) == 0
    m2 = (sub & 2) == 0
    for a in range(4):
        for j2 in range(2):
            Z = [U[b][(a * 2 + j2) * 8:(a * 2 + j2 + 1) * 8] for b in range(8)]
            for bit, s, m in ((2, 4, m4), (1, 2, m2)):
                for b in range(8):
                    if b & bit == 0:
                        A, B = Z[b], Z[b | bit]
                        Z[b] = jnp.where(m, A, pltpu.roll(B, s, 0))
                        Z[b | bit] = jnp.where(m, pltpu.roll(A, 8 - s, 0), B)
            for b in range(8):
                b2, j1, j0 = b >> 2, (b >> 1) & 1, b & 1
                out[j2 * 4 + j1 * 2 + j0][a * 2 + b2] = Z[b]
    return [jnp.concatenate(o, 0) for o in out]


def _kernel(x_hbm, wqkv_hbm, wo_hbm, w1_hbm, w3_hbm, w2_hbm, c_hbm, wmod_hbm, o_hbm,
            xv, wraw, wp, xh, cb, wo_raw, wo, w1, w3, w2, cv, wmod, mod,
            hA, hB, hS, kA, kB, kC, vA, vB, vC, qA, qB, qC, oA, oB, x1buf, h2buf, outv, sems, osems):
    NB = S // T
    globals_prg = PRG
    plan = {}

    def add(name, src, dst):
        plan[name] = pltpu.make_async_copy(src, dst, sems.at[len(plan)])

    def cols(ref, a, n):
        return ref.at[:, pl.ds(a, n)]

    def rows(ref, a, n):
        return ref.at[pl.ds(a, n), :]

    kofs = [sum(KCH[:i]) for i in range(len(KCH))]
    assert sum(KCH) == D
    add("c", c_hbm, cv)
    for q, (k0, kn) in enumerate(zip(kofs, KCH)):
        add(f"ms{q}", cols(wmod_hbm, k0, kn), cols(wmod, k0, kn))
        add(f"mc{q}", cols(wmod_hbm, D + k0, kn), cols(wmod, D + k0, kn))
        add(f"wq{q}", rows(wqkv_hbm, k0, kn), rows(wraw, k0, kn))
        if q == 0:
            add("x0", rows(x_hbm, 0, T), rows(xv, 0, T))
            add("x1", rows(x_hbm, T, T), rows(xv, T, T))
    add("x2", rows(x_hbm, 2 * T, 2 * T), rows(xv, 2 * T, 2 * T))
    add("wo", wo_hbm, wo_raw)
    add("mga", cols(wmod_hbm, 2 * D, D), cols(wmod, 2 * D, D))
    add("xr", rows(x_hbm, 4 * T, S - 4 * T), rows(xv, 4 * T, S - 4 * T))
    add("mb", cols(wmod_hbm, 3 * D, 3 * D), cols(wmod, 3 * D, 3 * D))
    add("w1", w1_hbm, w1)
    add("w3", w3_hbm, w3)
    add("w2", w2_hbm, w2)
    for d in plan.values():
        d.start()

    def need(name):
        plan[name].wait()

    need("c")
    cc = cv[...].astype(f32)
    sc = jnp.broadcast_to(cc * jax.nn.sigmoid(cc), (8, D)).astype(bf16)
    pred = (pltpu.bitcast(jnp.broadcast_to(cc[:, 0:128], (8, 128)), jnp.int32) | 1) != 0

    def gate(val, y):
        if y is None:
            return val
        return jnp.where(pred, jnp.full((8, 128), val, f32), y)

    def ld16(ref, idx):
        return pltpu.bitcast(ref[idx], bf16)

    def st16(ref, idx, val):
        ref[idx] = pltpu.bitcast(val.astype(bf16), u32)

    if VMOD or VMODB:
        cb[...] = jnp.broadcast_to(sc[0:1, :].astype(f32), (128, D)).T

    def mod_tile(c0, g=None):
        acc = None
        for r in range(0, D, 128):
            p = wmod[r:r + 128, c0:c0 + 128].astype(f32) * cb[r:r + 128, :]
            p = jnp.sum(p.reshape(16, 8, 128), axis=0)
            acc = p if acc is None else acc + p
        y = jnp.sum(acc, axis=0, keepdims=True)
        mod[0:1, c0:c0 + 128] = y
        return y

    for j in range(NT):
        kA[j, 0:HALO, :] = jnp.zeros((HALO, 128), f32)
        vA[j, 0:HALO, :] = jnp.zeros((HALO, 128), f32)

    Hs = (hA, hB); Ks = (kA, kB, kC); Vs = (vA, vB, vC); Qs = (qA, qB, qC); Os = (oA, oB)
    qscale = DH ** -0.5 * math.log2(math.e)

    def ln_rows(src, dst, r_src, r_dst2, rn, c_scale, c_shift, g):
        x = src[pl.ds(r_src, rn), :].astype(f32)
        sm = jnp.sum(x, axis=-1, keepdims=True)
        if g is None:
            m = sm * (1.0 / D)
        else:
            gv = gate(1.0 / D, g)
            m = sm * jnp.concatenate([gv] * (rn // 8), axis=0)[:, 0:1]
        xc = x - m
        v = jnp.mean(xc * xc, axis=-1, keepdims=True)
        hh = xc * lax.rsqrt(v + EPS) * (1.0 + mod[0:1, c_scale:c_scale + D]) + mod[0:1, c_shift:c_shift + D]
        st16(dst, (pl.ds(r_dst2, rn // 2), slice(None)), hh)

    def ln1_piece(i, q, g):
        rn = T // LNP
        ln_rows(xv, Hs[i % 2], i * T + q * rn, q * rn // 2, rn, D, 0, g)

    def ln2_piece(i, q, g):
        rn = T // LNP
        ln_rows(x1buf, h2buf, i * T + q * rn, (i * T + q * rn) // 2, rn, 4 * D, 3 * D, g)

    def xhat(blk, wait=True):
        if wait:
            need(f"x{blk}")
        rn = T // LN0P
        for p in range(LN0P):
            rs = slice(blk * T + p * rn, blk * T + (p + 1) * rn)
            x0 = xv[rs, :].astype(f32)
            xc = x0 - jnp.mean(x0, axis=-1, keepdims=True)
            xh[rs, :] = xc * lax.rsqrt(jnp.mean(xc * xc, axis=-1, keepdims=True) + EPS)

    modc = {}

    def mod_s(q):
        k0, kn = kofs[q], KCH[q]
        if VMOD:
            modc[q] = jnp.concatenate([mod_tile(k0 + t) for t in range(0, kn, 128)], axis=1)
        else:
            sa = jnp.dot(sc, wmod[:, k0:k0 + kn], preferred_element_type=f32)
            mod[:, k0:k0 + kn] = sa
            modc[q] = sa[0:1, :]

    def mod_c(q):
        k0, kn = kofs[q], KCH[q]
        if VMOD:
            ca = jnp.concatenate([mod_tile(D + k0 + t) for t in range(0, kn, 128)], axis=1)
        else:
            ca = jnp.dot(sc, wmod[:, D + k0:D + k0 + kn], preferred_element_type=f32)
            mod[:, D + k0:D + k0 + kn] = ca
            ca = ca[0:1, :]
        modc[q] = (modc[q], 1.0 + ca)

    def h_chunk(q, blk):
        k0, kn = kofs[q], KCH[q]
        sa, ca1 = modc[q]
        st16(hS, (slice(blk * T // 2, (blk + 1) * T // 2), slice(k0, k0 + kn)), xh[blk * T:(blk + 1) * T, k0:k0 + kn] * ca1 + sa)

    def prep(q, m, g=None):
        k0, kn = kofs[q], KCH[q]
        PRG = PRG0 if q == 0 else globals_prg
        lane = None
        if g is not None and GATEP:
            z = pltpu.bitcast(gate(0.0, g), jnp.int32)
            lane = lax.broadcasted_iota(jnp.int32, (PRG // 2, 128), 1) + jnp.concatenate([z] * (PRG // 16), axis=0)
        for r in range(k0, k0 + kn, PRG):
            X = [pltpu.bitcast(wraw[r:r + PRG, m * D + j * 128:m * D + (j + 1) * 128], u32) for j in range(NT)]
            X = _butterfly(X, lane)
            for j in range(NT):
                wp[r // 2:(r + PRG) // 2, m * D + j * 128:m * D + (j + 1) * 128] = X[j]

    def mm(q, blk, m):
        k0, kn = kofs[q], KCH[q]
        h = ld16(hS, (slice(blk * T // 2, (blk + 1) * T // 2), slice(k0, k0 + kn)))
        bufs, r0 = ((Qs, 0), (Ks, HALO), (Vs, HALO))[m]
        y = jnp.dot(h, ld16(wp, (slice(k0 // 2, (k0 + kn) // 2), slice(m * D, (m + 1) * D))), preferred_element_type=f32)
        dst = bufs[blk]
        for j in range(NT):
            if q == 0:
                dst[j, r0:r0 + T, :] = y[:, j * 128:(j + 1) * 128]
            else:
                dst[j, r0:r0 + T, :] = dst[j, r0:r0 + T, :] + y[:, j * 128:(j + 1) * 128]
        return y[T - 8:T, D - 128:D]

    NQ = len(KCH)
    with scope("s1_a0"):
        need("ms0"); need("mc0")
        mod_s(0); mod_c(0)
        need("wq0")
        for m in range(3):
            prep(0, m)
        xhat(0)
        h_chunk(0, 0)
    mx = [functools.partial(mm, 0, 0, m) for m in range(3)] + [functools.partial(mm, 0, 1, m) for m in range(3)]
    mx += [functools.partial(mm, q, blk, m) for q in range(1, NQ) for m in range(3) for blk in range(2)]
    after = {}
    def at(pos, fn):
        after.setdefault(pos, []).append(fn)
    for q in range(1, NQ):
        ex = min((q - 1) * OFFGROW, OFFMAX - OFF_W)
        at(6 * q - OFF_W - ex - 1, lambda g, q=q: (need(f"ms{q}"), need(f"mc{q}"), need(f"wq{q}")))
        at(6 * q - OFF_W - ex, lambda g, q=q: mod_s(q))
        at(6 * q - OFF_C - ex, lambda g, q=q: mod_c(q))
        at(6 * q - OFF_H - ex, lambda g, q=q: (h_chunk(q, 0), h_chunk(q, 1)))
        for m in range(3):
            at(6 * q - OFF_P[m] - ex, lambda g, q=q, m=m: prep(q, m, g))
    at(0, lambda g: need("x1"))
    for p in range(LNP):
        at(6 * NQ - 6 + (5 * p) // LNP, lambda g, p=p: ln1_piece(2, p, g))
    at(6 * NQ - 7, lambda g: need("x2"))
    at(1, lambda g: (xhat(1, False), h_chunk(0, 1)))
    for e, item in enumerate(mx):
        y = item()
        for fn in after.get(e, []):
            fn(y)
    for j in range(NT):
        Ks[1][j, 0:HALO, :] = Ks[0][j, T:T + HALO, :]
        Vs[1][j, 0:HALO, :] = Vs[0][j, T:T + HALO, :]

    def attn_chunk(i, c, g):
        qbuf, k_ref, v_ref, obuf = Qs[i % 3], Ks[i % 3], Vs[i % 3], Os[i % 2]
        rs = slice(c * RC, (c + 1) * RC)
        sg = gate(qscale, g)
        if g is not None and RC > 8:
            sg = jnp.concatenate([sg] * (RC // 8), axis=0)
        qt = [qbuf[j, rs, :] * sg for j in range(NT)]
        ls = []
        for w in range(W):
            o = HALO - DIL * w + c * RC
            s = None
            for j in range(NT):
                p = qt[j] * k_ref[j, o:o + RC, :]
                s = p if s is None else s + p
            s = _group_allreduce(s)
            if i == 0 and c * RC < DIL * w:
                row = c * RC + lax.broadcasted_iota(jnp.int32, (RC, 128), 0)
                s = jnp.where(row >= DIL * w, s, -1.5e9)
            ls.append(s)
        m = functools.reduce(jnp.maximum, ls)
        es = [jnp.exp2(l - m) for l in ls]
        r = 1.0 / functools.reduce(jnp.add, es)
        ps = [e * r for e in es]
        for j in range(NT):
            acc = None
            for w in range(W):
                o = HALO - DIL * w + c * RC
                p = ps[w] * v_ref[j, o:o + RC, :]
                acc = p if acc is None else acc + p
            obuf[rs, j * 128:(j + 1) * 128] = acc.astype(bf16)

    def qkv_items(i):
        p, pp = i % 3, (i - 1) % 3
        st = {}
        def mk(n):
            def run():
                if n == 0:
                    for j in range(NT):
                        Ks[p][j, 0:HALO, :] = Ks[pp][j, T:T + HALO, :]
                        Vs[p][j, 0:HALO, :] = Vs[pp][j, T:T + HALO, :]
                    st["h"] = pltpu.bitcast(Hs[i % 2][...], bf16)
                y = jnp.dot(st["h"], ld16(wp, (slice(None), slice(n * 128, (n + 1) * 128))), preferred_element_type=f32)
                dst, r0 = ((Qs[p], 0), (Ks[p], HALO), (Vs[p], HALO))[n // NT]
                dst[n % NT, r0:r0 + T, :] = y
                return y[T - 8:T, :]
            return run
        return [mk(n) for n in range(3 * NT)]

    def wo_items(i):
        st = {}
        def mk(n):
            def run():
                if n == 0:
                    st["o"] = Os[i % 2][...]
                cs = slice(n * 128, (n + 1) * 128)
                a = jnp.dot(st["o"], ld16(wo, (slice(None), cs)), preferred_element_type=f32)
                x1buf[i * T:(i + 1) * T, cs] = xv[i * T:(i + 1) * T, cs].astype(f32) + mod[0:1, 2 * D + n * 128:2 * D + (n + 1) * 128] * a
                return a[T - 8:T, :]
            return run
        return [mk(n) for n in range(NT)]

    def ffn_coarse(i, r0, h):
        acc = None
        for f in range(F // FC):
            fs = slice(f * FC, (f + 1) * FC)
            g = jnp.dot(h, w1[:, fs], preferred_element_type=f32)
            u = jnp.dot(h, w3[:, fs], preferred_element_type=f32)
            a = (g * jax.nn.sigmoid(g) * u).astype(bf16)
            d = jnp.dot(a, w2[fs, :], preferred_element_type=f32)
            acc = d if acc is None else acc + d
        ffn_fin(i, r0, acc)

    def ffn_fin(i, r0, acc):
        outv[pl.ds(r0, T), :] = (x1buf[pl.ds(r0, T), :] + mod[0:1, 5 * D:6 * D] * acc).astype(bf16)
        pltpu.make_async_copy(outv.at[pl.ds(r0, T), :], o_hbm.at[pl.ds(r0, T), :], osems.at[i]).start()

    def ffn_items(i, r0):
        st = {"acc": [None] * NT, "g": {}, "u": {}, "h": None, "a": {}}
        items = []
        nt = FC // 128
        def gu(f, t, which):
            def run():
                if st["h"] is None:
                    st["h"] = pltpu.bitcast(h2buf[r0 // 2:(r0 + T) // 2, :], bf16)
                cs = slice(f * FC + t * 128, f * FC + (t + 1) * 128)
                y = jnp.dot(st["h"], (w1 if which == "g" else w3)[:, cs], preferred_element_type=f32)
                st[which][(f, t)] = y
                if which == "u":
                    g = st["g"].pop((f, t)); u = st["u"].pop((f, t))
                    st["a"][(f, t)] = (g * jax.nn.sigmoid(g) * u).astype(bf16)
                return y[T - 8:T, :]
            return run
        def dn(f, n):
            def run():
                if n == 0:
                    st["af"] = jnp.concatenate([st["a"].pop((f, t)) for t in range(nt)], axis=1)
                d = jnp.dot(st["af"], w2[f * FC:(f + 1) * FC, n * 128:(n + 1) * 128], preferred_element_type=f32)
                st["acc"][n] = d if st["acc"][n] is None else st["acc"][n] + d
                return d[T - 8:T, :]
            return run
        per_f = []
        for f in range(F // FC):
            it = []
            for t in range(nt):
                it += [gu(f, t, "g"), gu(f, t, "u")]
            it += [dn(f, n) for n in range(NT)]
            per_f.append(it)
        def fin():
            ffn_fin(i, r0, jnp.concatenate(st["acc"], axis=1))
            return None
        return per_f, fin

    def run_paced(mx, vec, wts=None):
        wts = wts or [1.0] * len(mx)
        tot = sum(wts)
        vec = sorted(vec, key=lambda t: t[0])
        vi = 0
        cum = 0.0
        for e, item in enumerate(mx):
            y = item()
            cum += wts[e]
            while vi < len(vec) and vec[vi][0] * tot < cum:
                vec[vi][1](y); vi += 1
        while vi < len(vec):
            vec[vi][1](None); vi += 1

    NC = T // RC

    def att_vec(i, lo=0.0, span=None):
        span = ASPAN if span is None else span
        return [(lo + span * c / NC, functools.partial(attn_chunk, i, c)) for c in range(NC)]

    def ln1_vec(i, lo, span):
        return [(lo + span * q / LNP, functools.partial(ln1_piece, i, q)) for q in range(LNP)]

    def ln2_vec(i, lo, span):
        return [(lo + span * q / LNP, functools.partial(ln2_piece, i, q)) for q in range(LNP)]

    def wo_prep(cb, g):
        X = [wo_raw[b * 128:(b + 1) * 128, cb * 128:(cb + 1) * 128] for b in range(NT)]
        Y = _rowperm(X)
        for j in range(NT):
            wo[j * 64:(j + 1) * 64, cb * 128:(cb + 1) * 128] = Y[j]

    def mod_item(name, c0, cn):
        def run():
            if name:
                need(name)
            y = jnp.dot(sc, wmod[:, c0:c0 + cn], preferred_element_type=f32)
            mod[:, c0:c0 + cn] = y
            return y[:, 0:128]
        return run

    tail_f, tail_fin = ffn_items(0, 0)
    for i in range(0, NB + 1):
        with scope(f"s3_body{i}"):
            mx, vec, wts = [], [], []
            def addmx(items, w=1.0):
                mx.extend(items); wts.extend([w] * len(items))
            if i == NB - 2:
                need("w1"); need("w3"); need("w2")
            if i == 1:
                need("wo"); need("mga"); need("xr")
                addmx(qkv_items(i + 2))
                addmx(wo_items(i - 1))
                vec += [(0.1 + 0.5 * cb / NT, functools.partial(wo_prep, cbi)) for cb, cbi in enumerate(range(NT))]
                vec += [(0.12 + 0.5 * t / NT, functools.partial(mod_tile, 2 * D + t * 128)) for t in range(NT)]
            else:
                if i >= 1:
                    addmx(wo_items(i - 1))
                if i + 2 < NB:
                    addmx(qkv_items(i + 2))
            if i == 2:
                need("mb")
            if VMODB:
                if 2 <= i <= 4:
                    vec += [(0.05 + 0.9 * t / NT, functools.partial(mod_tile, (1 + i) * D + t * 128)) for t in range(NT)]
            elif i == MODB_AT:
                addmx([mod_item(None, 3 * D + t * 512, 512) for t in range(6)], 0.5)
            if i < NB:
                vec += att_vec(i, span=(ASPAN if i < NB - 2 else TSPAN))
            if i + 3 < NB:
                vec += ln1_vec(i + 3, LNOFF / 32, LSPAN)
            if i == 5:
                vec += ln2_vec(0, 0.05, 0.4)
            if i == 5:
                vec += ln2_vec(1, 0.5, 0.4)
            if i == NB - 2:
                for f in range(TAILSPLIT):
                    addmx(tail_f[f])
            if i == NB - 1:
                for f in range(TAILSPLIT, F // FC):
                    addmx(tail_f[f])
                addmx([tail_fin], 0.0)
            run_paced(mx, vec, wts)

    def ffn(i, has_next):
        static = isinstance(i, int)
        r0 = i * T if static else pl.multiple_of(i * T, T)
        p0 = i * (T // 2) if static else pl.multiple_of(i * (T // 2), T // 2)
        h = pltpu.bitcast(h2buf[pl.ds(p0, T // 2), :], bf16)
        if has_next:
            ln_rows(x1buf, h2buf, r0 + T, p0 + T // 2, T, 4 * D, 3 * D, None)
        ffn_coarse(i, r0, h)

    with scope("s4_loop"):
        lax.fori_loop(1, NB - 1, lambda i, c: (ffn(i, True), 0)[1], 0)
    with scope("s5_last"):
        ffn(NB - 1, False)
    for i in range(NB):
        pltpu.make_async_copy(outv.at[pl.ds(i * T, T), :], o_hbm.at[pl.ds(i * T, T), :], osems.at[i]).wait()


def pallas_adaLN_cond__sliding_local_dilated__glu_gated_swiglu__prompt_kernel(
        A_x, A_wqkv, A_wo, B_x, B_w1, B_w3, B_w2, c, w_mod):
    NB = S // T
    anyspec = pl.BlockSpec(memory_space=pl.ANY)
    kv_shape = pltpu.VMEM((NT, T + HALO, 128), f32)
    flags = {"XLA_TPU_EVENLY_DISTRIBUTE_CRITICAL_NODES": True} if EVEN else {}
    out = pl.pallas_call(
        _kernel,
        out_shape=jax.ShapeDtypeStruct((S, D), bf16),
        in_specs=[anyspec] * 8,
        out_specs=anyspec,
        scratch_shapes=[
            pltpu.VMEM((S, D), bf16),
            pltpu.VMEM((D, 3 * D), bf16),
            pltpu.VMEM((D // 2, 3 * D), u32),
            pltpu.VMEM((2 * T, D), f32),
            pltpu.VMEM((D, 128), f32),
            pltpu.VMEM((D, D), bf16),
            pltpu.VMEM((D // 2, D), u32),
            pltpu.VMEM((D, F), bf16),
            pltpu.VMEM((D, F), bf16),
            pltpu.VMEM((F, D), bf16),
            pltpu.VMEM((1, D), bf16),
            pltpu.VMEM((D, 6 * D), bf16),
            pltpu.VMEM((8, 6 * D), f32),
            pltpu.VMEM((T // 2, D), u32), pltpu.VMEM((T // 2, D), u32), pltpu.VMEM((T, D), u32),
            kv_shape, kv_shape, kv_shape, kv_shape, kv_shape, kv_shape,
            pltpu.VMEM((NT, T, 128), f32), pltpu.VMEM((NT, T, 128), f32), pltpu.VMEM((NT, T, 128), f32),
            pltpu.VMEM((T, D), bf16), pltpu.VMEM((T, D), bf16),
            pltpu.VMEM((S, D), f32),
            pltpu.VMEM((S // 2, D), u32),
            pltpu.VMEM((S, D), bf16),
            pltpu.SemaphoreType.DMA((40,)),
            pltpu.SemaphoreType.DMA((NB,)),
        ],
        compiler_params=pltpu.CompilerParams(vmem_limit_bytes=120 * 1024 * 1024, flags=flags),
    )(A_x.reshape(S, D), A_wqkv, A_wo, B_w1, B_w3, B_w2, c, w_mod)
    return out.reshape(1, S, D)
```

```python
import contextlib
import functools
import math
import jax
import jax.numpy as jnp
import numpy as np
from jax import lax
from jax.experimental import pallas as pl
from jax.experimental.pallas import tpu as pltpu

S, D, F, H, DH, W, DIL = 2048, 1024, 3584, 32, 32, 8, 2
EPS = 1e-5
T = 256
FC = 512
HALO = 16
NT = D // 128
RC = 8
KCH = (128,) * 8
PRG = 64
PRG0 = 128
OFF_W = 3
OFF_C = 2
OFF_H = 2
OFF_P = (3, 1, -1)
OFFGROW = 1
OFFMAX = 6
ONEDOT = False
WAITS = ((2, (1,)), (7, (2,)), (12, (3,)), (17, (4,)), (23, (5,)), (29, (6,)), (35, (7,)))
VMODGA = False
MODP = 4
PEEL = False
START2 = True
LN2P = 0
X1AT = 1
VMOD = False
VMODB = False
HALFW = True
LN0P = 4
ASPAN = 0.875
LSPAN = 0.75
LNP = 8
LNOFF = 1
TAILSPLIT = 3
TSPAN = 0.9
MODB_AT = 3
WOPREP = 0.3
EVEN = True
SCOPES = False
XSPLIT = True
GATEP = False
f32, bf16, u32 = jnp.float32, jnp.bfloat16, jnp.uint32


def scope(name):
    return jax.named_scope(name) if SCOPES else contextlib.nullcontext()


def _group_allreduce(s):
    lane = lax.broadcasted_iota(jnp.int32, s.shape, 1)
    s = s + jnp.where((lane & 1) == 0, pltpu.roll(s, 127, 1), pltpu.roll(s, 1, 1))
    s = s + jnp.where((lane & 2) == 0, pltpu.roll(s, 126, 1), pltpu.roll(s, 2, 1))
    return s


def _butterfly(X, lane=None):
    X = list(X)
    if lane is None:
        lane = lax.broadcasted_iota(jnp.int32, X[0].shape, 1)
    for b, s in ((1, 4), (2, 8), (4, 16)):
        m = (lane & s) == 0
        for i in range(NT):
            if i & b == 0:
                A, B = X[i], X[i | b]
                X[i] = jnp.where(m, A, pltpu.roll(B, s, 1))
                X[i | b] = jnp.where(m, pltpu.roll(A, 128 - s, 1), B)
    return X


def _rowperm(X):
    C = X[0].shape[1]
    U = [pltpu.bitcast(x, u32) for x in X]
    out = [[None] * 8 for _ in range(8)]
    sub = lax.broadcasted_iota(jnp.int32, (8, C), 0)
    m4 = (sub & 4) == 0
    m2 = (sub & 2) == 0
    for a in range(4):
        for j2 in range(2):
            Z = [U[b][(a * 2 + j2) * 8:(a * 2 + j2 + 1) * 8] for b in range(8)]
            for bit, s, m in ((2, 4, m4), (1, 2, m2)):
                for b in range(8):
                    if b & bit == 0:
                        A, B = Z[b], Z[b | bit]
                        Z[b] = jnp.where(m, A, pltpu.roll(B, s, 0))
                        Z[b | bit] = jnp.where(m, pltpu.roll(A, 8 - s, 0), B)
            for b in range(8):
                b2, j1, j0 = b >> 2, (b >> 1) & 1, b & 1
                out[j2 * 4 + j1 * 2 + j0][a * 2 + b2] = Z[b]
    return [jnp.concatenate(o, 0) for o in out]


def _kernel(x_hbm, wqkv_hbm, wo_hbm, w1_hbm, w3_hbm, w2_hbm, c_hbm, wmod_hbm, o_hbm,
            xv, wraw, wp, xh, cb, wo_raw, wo, w1, w3, w2, cv, wmod, mod,
            hA, hB, hS, kA, kB, kC, vA, vB, vC, qA, qB, qC, oA, oB, x1buf, h2buf, h2nxt, outv, sems, osems):
    NB = S // T
    globals_prg = PRG
    plan = {}

    def add(name, src, dst):
        plan[name] = pltpu.make_async_copy(src, dst, sems.at[len(plan)])

    def cols(ref, a, n):
        return ref.at[:, pl.ds(a, n)]

    def rows(ref, a, n):
        return ref.at[pl.ds(a, n), :]

    kofs = [sum(KCH[:i]) for i in range(len(KCH))]
    assert sum(KCH) == D
    add("c", c_hbm, cv)
    for q, (k0, kn) in enumerate(zip(kofs, KCH)):
        add(f"ms{q}", cols(wmod_hbm, k0, kn), cols(wmod, k0, kn))
        add(f"mc{q}", cols(wmod_hbm, D + k0, kn), cols(wmod, D + k0, kn))
        if q == 0 and START2:
            add("x0", rows(x_hbm, 0, T), rows(xv, 0, T))
            for m in range(3):
                add(f"wq0{m}", wqkv_hbm.at[pl.ds(k0, kn), pl.ds(m * D, D)], wraw.at[pl.ds(k0, kn), pl.ds(m * D, D)])
            add("x1", rows(x_hbm, T, T), rows(xv, T, T))
            continue
        add(f"wq{q}", rows(wqkv_hbm, k0, kn), rows(wraw, k0, kn))
        if q == 0:
            add("x0", rows(x_hbm, 0, T), rows(xv, 0, T))
            add("x1", rows(x_hbm, T, T), rows(xv, T, T))
    add("x2", rows(x_hbm, 2 * T, 2 * T), rows(xv, 2 * T, 2 * T))
    add("wo", wo_hbm, wo_raw)
    add("mga", cols(wmod_hbm, 2 * D, D), cols(wmod, 2 * D, D))
    add("xr", rows(x_hbm, 4 * T, S - 4 * T), rows(xv, 4 * T, S - 4 * T))
    add("mb", cols(wmod_hbm, 3 * D, 3 * D), cols(wmod, 3 * D, 3 * D))
    add("w1", w1_hbm, w1)
    add("w3", w3_hbm, w3)
    add("w2", w2_hbm, w2)
    for d in plan.values():
        d.start()

    def need(name):
        plan[name].wait()

    need("c")
    cc = cv[...].astype(f32)
    sc = jnp.broadcast_to(cc * jax.nn.sigmoid(cc), (8, D)).astype(bf16)
    pred = (pltpu.bitcast(jnp.broadcast_to(cc[:, 0:128], (8, 128)), jnp.int32) | 1) != 0

    def gate(val, y):
        if y is None:
            return val
        return jnp.where(pred, jnp.full((8, 128), val, f32), y)

    def ld16(ref, idx):
        return pltpu.bitcast(ref[idx], bf16)

    def st16(ref, idx, val):
        ref[idx] = pltpu.bitcast(val.astype(bf16), u32)

    if VMOD or VMODB or VMODGA:
        cb[...] = jnp.broadcast_to(sc[0:1, :].astype(f32), (128, D)).T

    def mod_tile(c0, g=None):
        acc = None
        for r in range(0, D, 128):
            p = wmod[r:r + 128, c0:c0 + 128].astype(f32) * cb[r:r + 128, :]
            p = jnp.sum(p.reshape(16, 8, 128), axis=0)
            acc = p if acc is None else acc + p
        y = jnp.sum(acc, axis=0, keepdims=True)
        mod[0:1, c0:c0 + 128] = y
        return y

    modst = {}

    def mod_piece(c0, p, g=None):
        rn = D // MODP
        acc = modst.get(c0)
        for r in range(p * rn, (p + 1) * rn, 128):
            t = wmod[r:r + 128, c0:c0 + 128].astype(f32) * cb[r:r + 128, :]
            t = jnp.sum(t.reshape(16, 8, 128), axis=0)
            acc = t if acc is None else acc + t
        if p == MODP - 1:
            mod[0:1, c0:c0 + 128] = jnp.sum(acc, axis=0, keepdims=True)
            modst.pop(c0, None)
        else:
            modst[c0] = acc

    def mod_vec(cols0, lo, span):
        items = [(c0, p) for c0 in cols0 for p in range(MODP)]
        return [(lo + span * n / len(items), functools.partial(mod_piece, c0, p)) for n, (c0, p) in enumerate(items)]

    for j in range(NT):
        kA[j, 0:HALO, :] = jnp.zeros((HALO, 128), f32)
        vA[j, 0:HALO, :] = jnp.zeros((HALO, 128), f32)

    Hs = (hA, hB); Ks = (kA, kB, kC); Vs = (vA, vB, vC); Qs = (qA, qB, qC); Os = (oA, oB)
    qscale = DH ** -0.5 * math.log2(math.e)

    def ln_rows(src, dst, r_src, r_dst2, rn, c_scale, c_shift, g):
        x = src[pl.ds(r_src, rn), :].astype(f32)
        sm = jnp.sum(x, axis=-1, keepdims=True)
        if g is None:
            m = sm * (1.0 / D)
        else:
            gv = gate(1.0 / D, g)
            m = sm * jnp.concatenate([gv] * (rn // 8), axis=0)[:, 0:1]
        xc = x - m
        v = jnp.mean(xc * xc, axis=-1, keepdims=True)
        hh = xc * lax.rsqrt(v + EPS) * (1.0 + mod[0:1, c_scale:c_scale + D]) + mod[0:1, c_shift:c_shift + D]
        st16(dst, (pl.ds(r_dst2, rn // 2), slice(None)), hh)

    def ln1_piece(i, q, g):
        rn = T // LNP
        ln_rows(xv, Hs[i % 2], i * T + q * rn, q * rn // 2, rn, D, 0, g)

    def ln2_piece(i, q, g):
        rn = T // LNP
        ln_rows(x1buf, h2buf, i * T + q * rn, (i * T + q * rn) // 2, rn, 4 * D, 3 * D, g)

    def xhat(blk, wait=True):
        if wait:
            need(f"x{blk}")
        rn = T // LN0P
        for p in range(LN0P):
            rs = slice(blk * T + p * rn, blk * T + (p + 1) * rn)
            x0 = xv[rs, :].astype(f32)
            xc = x0 - jnp.mean(x0, axis=-1, keepdims=True)
            xh[rs, :] = xc * lax.rsqrt(jnp.mean(xc * xc, axis=-1, keepdims=True) + EPS)

    modc = {}

    def mod_s(q):
        k0, kn = kofs[q], KCH[q]
        if VMOD:
            modc[q] = jnp.concatenate([mod_tile(k0 + t) for t in range(0, kn, 128)], axis=1)
        else:
            sa = jnp.dot(sc, wmod[:, k0:k0 + kn], preferred_element_type=f32)
            mod[:, k0:k0 + kn] = sa
            modc[q] = sa[0:1, :]

    def mod_c(q):
        k0, kn = kofs[q], KCH[q]
        if VMOD:
            ca = jnp.concatenate([mod_tile(D + k0 + t) for t in range(0, kn, 128)], axis=1)
        else:
            ca = jnp.dot(sc, wmod[:, D + k0:D + k0 + kn], preferred_element_type=f32)
            mod[:, D + k0:D + k0 + kn] = ca
            ca = ca[0:1, :]
        modc[q] = (modc[q], 1.0 + ca)

    def h_chunk(q, blk):
        k0, kn = kofs[q], KCH[q]
        sa, ca1 = modc[q]
        st16(hS, (slice(blk * T // 2, (blk + 1) * T // 2), slice(k0, k0 + kn)), xh[blk * T:(blk + 1) * T, k0:k0 + kn] * ca1 + sa)

    def prep(q, m, g=None):
        k0, kn = kofs[q], KCH[q]
        PRG = PRG0 if q == 0 else globals_prg
        lane = None
        if g is not None and GATEP:
            z = pltpu.bitcast(gate(0.0, g), jnp.int32)
            lane = lax.broadcasted_iota(jnp.int32, (PRG // 2, 128), 1) + jnp.concatenate([z] * (PRG // 16), axis=0)
        for r in range(k0, k0 + kn, PRG):
            X = [pltpu.bitcast(wraw[r:r + PRG, m * D + j * 128:m * D + (j + 1) * 128], u32) for j in range(NT)]
            X = _butterfly(X, lane)
            for j in range(NT):
                wp[r // 2:(r + PRG) // 2, m * D + j * 128:m * D + (j + 1) * 128] = X[j]

    def mm(q, blk, m):
        k0, kn = kofs[q], KCH[q]
        h = ld16(hS, (slice(blk * T // 2, (blk + 1) * T // 2), slice(k0, k0 + kn)))
        bufs, r0 = ((Qs, 0), (Ks, HALO), (Vs, HALO))[m]
        y = jnp.dot(h, ld16(wp, (slice(k0 // 2, (k0 + kn) // 2), slice(m * D, (m + 1) * D))), preferred_element_type=f32)
        dst = bufs[blk]
        for j in range(NT):
            if q == 0:
                dst[j, r0:r0 + T, :] = y[:, j * 128:(j + 1) * 128]
            else:
                dst[j, r0:r0 + T, :] = dst[j, r0:r0 + T, :] + y[:, j * 128:(j + 1) * 128]
        return y[T - 8:T, D - 128:D]

    NQ = len(KCH)
    with scope("s1_a0"):
        need("ms0"); need("mc0")
    if START2:
        with scope("s1_a1"):
            mod_s(0); mod_c(0)
            need("x0")
        with scope("s1_a2"):
            xhat(0, False)
            h_chunk(0, 0)
            need("wq00")
        with scope("s1_a3"):
            prep(0, 0)
            need("wq01")
    else:
        with scope("s1_a1"):
            mod_s(0); mod_c(0)
            need("wq0")
        with scope("s1_a2"):
            for m in range(3):
                prep(0, m)
            need("x0")
        with scope("s1_a3"):
            xhat(0, False)
            h_chunk(0, 0)
    mx = [functools.partial(mm, 0, 0, m) for m in range(3)] + [functools.partial(mm, 0, 1, m) for m in range(3)]
    mx += [functools.partial(mm, q, blk, m) for q in range(1, NQ) for m in range(3) for blk in range(2)]
    after = {}
    def at(pos, fn):
        after.setdefault(pos, []).append(fn)
    for q in range(1, NQ):
        ex = min((q - 1) * OFFGROW, OFFMAX - OFF_W)
        at(6 * q - OFF_W - ex, lambda g, q=q: mod_s(q))
        at(6 * q - OFF_C - ex, lambda g, q=q: mod_c(q))
        at(6 * q - OFF_H - ex, lambda g, q=q: (h_chunk(q, 0), h_chunk(q, 1)))
        for m in range(3):
            at(6 * q - OFF_P[m] - ex, lambda g, q=q, m=m: prep(q, m, g))
    if START2:
        pre = {0: lambda: prep(0, 1), 1: lambda: prep(0, 2)}
        at(0, lambda g: need("wq02"))
        at(1, lambda g: need("x1"))
        at(2, lambda g: (xhat(1, False), h_chunk(0, 1)))
    else:
        pre = {}
        at(0, lambda g: need("x1"))
    waits = {}
    for pos, qs in WAITS:
        waits[pos] = qs
    for p in range(LNP):
        at(6 * NQ - 6 + (5 * p) // LNP, lambda g, p=p: ln1_piece(2, p, g))
    at(6 * NQ - 7, lambda g: need("x2"))
    if not START2:
        at(1, lambda g: (xhat(1, False), h_chunk(0, 1)))
    bounds = [0] + [p + 1 for p in sorted(waits)] + [len(mx)]
    for bi in range(len(bounds) - 1):
        with scope(f"s2_seg{bi:02d}_{bounds[bi]}"):
            for e in range(bounds[bi], bounds[bi + 1]):
                y = mx[e]()
                if e in pre:
                    pre[e]()
                for fn in after.get(e, []):
                    fn(y)
                for q in waits.get(e, ()):
                    need(f"ms{q}"); need(f"mc{q}"); need(f"wq{q}")
    for j in range(NT):
        Ks[1][j, 0:HALO, :] = Ks[0][j, T:T + HALO, :]
        Vs[1][j, 0:HALO, :] = Vs[0][j, T:T + HALO, :]

    def attn_chunk(i, c, g):
        qbuf, k_ref, v_ref, obuf = Qs[i % 3], Ks[i % 3], Vs[i % 3], Os[i % 2]
        rs = slice(c * RC, (c + 1) * RC)
        sg = gate(qscale, g)
        if g is not None and RC > 8:
            sg = jnp.concatenate([sg] * (RC // 8), axis=0)
        qt = [qbuf[j, rs, :] * sg for j in range(NT)]
        ls = []
        for w in range(W):
            o = HALO - DIL * w + c * RC
            s = None
            for j in range(NT):
                p = qt[j] * k_ref[j, o:o + RC, :]
                s = p if s is None else s + p
            s = _group_allreduce(s)
            if i == 0 and c * RC < DIL * w:
                row = c * RC + lax.broadcasted_iota(jnp.int32, (RC, 128), 0)
                s = jnp.where(row >= DIL * w, s, -1.5e9)
            ls.append(s)
        m = functools.reduce(jnp.maximum, ls)
        es = [jnp.exp2(l - m) for l in ls]
        r = 1.0 / functools.reduce(jnp.add, es)
        ps = [e * r for e in es]
        for j in range(NT):
            acc = None
            for w in range(W):
                o = HALO - DIL * w + c * RC
                p = ps[w] * v_ref[j, o:o + RC, :]
                acc = p if acc is None else acc + p
            obuf[rs, j * 128:(j + 1) * 128] = acc.astype(bf16)

    def qkv_items(i):
        p, pp = i % 3, (i - 1) % 3
        st = {}
        def mk(n):
            def run():
                if n == 0:
                    for j in range(NT):
                        Ks[p][j, 0:HALO, :] = Ks[pp][j, T:T + HALO, :]
                        Vs[p][j, 0:HALO, :] = Vs[pp][j, T:T + HALO, :]
                    st["h"] = pltpu.bitcast(Hs[i % 2][...], bf16)
                y = jnp.dot(st["h"], ld16(wp, (slice(None), slice(n * 128, (n + 1) * 128))), preferred_element_type=f32)
                dst, r0 = ((Qs[p], 0), (Ks[p], HALO), (Vs[p], HALO))[n // NT]
                dst[n % NT, r0:r0 + T, :] = y
                return y[T - 8:T, :]
            return run
        return [mk(n) for n in range(3 * NT)]

    def wo_items(i):
        st = {}
        def mk(n):
            def run():
                if n == 0:
                    st["o"] = Os[i % 2][...]
                cs = slice(n * 128, (n + 1) * 128)
                a = jnp.dot(st["o"], ld16(wo, (slice(None), cs)), preferred_element_type=f32)
                x1buf[i * T:(i + 1) * T, cs] = xv[i * T:(i + 1) * T, cs].astype(f32) + mod[0:1, 2 * D + n * 128:2 * D + (n + 1) * 128] * a
                return a[T - 8:T, :]
            return run
        return [mk(n) for n in range(NT)]

    def ffn_coarse(i, r0, h):
        acc = None
        for f in range(F // FC):
            fs = slice(f * FC, (f + 1) * FC)
            g = jnp.dot(h, w1[:, fs], preferred_element_type=f32)
            u = jnp.dot(h, w3[:, fs], preferred_element_type=f32)
            a = (g * jax.nn.sigmoid(g) * u).astype(bf16)
            d = jnp.dot(a, w2[fs, :], preferred_element_type=f32)
            acc = d if acc is None else acc + d
        ffn_fin(i, r0, acc)

    def ffn_fin(i, r0, acc):
        outv[pl.ds(r0, T), :] = (x1buf[pl.ds(r0, T), :] + mod[0:1, 5 * D:6 * D] * acc).astype(bf16)
        pltpu.make_async_copy(outv.at[pl.ds(r0, T), :], o_hbm.at[pl.ds(r0, T), :], osems.at[i]).start()

    def ffn_items(i, r0):
        st = {"acc": [None] * NT, "g": {}, "u": {}, "h": None, "a": {}}
        items = []
        nt = FC // 128
        def gu(f, t, which):
            def run():
                if st["h"] is None:
                    st["h"] = pltpu.bitcast(h2buf[r0 // 2:(r0 + T) // 2, :], bf16)
                cs = slice(f * FC + t * 128, f * FC + (t + 1) * 128)
                y = jnp.dot(st["h"], (w1 if which == "g" else w3)[:, cs], preferred_element_type=f32)
                st[which][(f, t)] = y
                if which == "u":
                    g = st["g"].pop((f, t)); u = st["u"].pop((f, t))
                    st["a"][(f, t)] = (g * jax.nn.sigmoid(g) * u).astype(bf16)
                return y[T - 8:T, :]
            return run
        def dn(f, n):
            def run():
                if n == 0:
                    st["af"] = jnp.concatenate([st["a"].pop((f, t)) for t in range(nt)], axis=1)
                d = jnp.dot(st["af"], w2[f * FC:(f + 1) * FC, n * 128:(n + 1) * 128], preferred_element_type=f32)
                st["acc"][n] = d if st["acc"][n] is None else st["acc"][n] + d
                return d[T - 8:T, :]
            return run
        per_f = []
        for f in range(F // FC):
            it = []
            for t in range(nt):
                it += [gu(f, t, "g"), gu(f, t, "u")]
            it += [dn(f, n) for n in range(NT)]
            per_f.append(it)
        def fin():
            ffn_fin(i, r0, jnp.concatenate(st["acc"], axis=1))
            return None
        return per_f, fin

    def run_paced(mx, vec, wts=None):
        wts = wts or [1.0] * len(mx)
        tot = sum(wts)
        vec = sorted(vec, key=lambda t: t[0])
        vi = 0
        cum = 0.0
        for e, item in enumerate(mx):
            y = item()
            cum += wts[e]
            while vi < len(vec) and vec[vi][0] * tot < cum:
                vec[vi][1](y); vi += 1
        while vi < len(vec):
            vec[vi][1](None); vi += 1

    NC = T // RC

    def att_vec(i, lo=0.0, span=None):
        span = ASPAN if span is None else span
        return [(lo + span * c / NC, functools.partial(attn_chunk, i, c)) for c in range(NC)]

    def ln1_vec(i, lo, span):
        return [(lo + span * q / LNP, functools.partial(ln1_piece, i, q)) for q in range(LNP)]

    def ln2_vec(i, lo, span):
        return [(lo + span * q / LNP, functools.partial(ln2_piece, i, q)) for q in range(LNP)]

    def wo_prep(cb, g):
        X = [wo_raw[b * 128:(b + 1) * 128, cb * 128:(cb + 1) * 128] for b in range(NT)]
        Y = _rowperm(X)
        for j in range(NT):
            wo[j * 64:(j + 1) * 64, cb * 128:(cb + 1) * 128] = Y[j]

    def mod_item(name, c0, cn):
        def run():
            if name:
                need(name)
            y = jnp.dot(sc, wmod[:, c0:c0 + cn], preferred_element_type=f32)
            mod[:, c0:c0 + cn] = y
            return y[:, 0:128]
        return run

    tail_f, tail_fin = ffn_items(0, 0)
    for i in range(0, NB + 1):
        with scope(f"s3_body{i}"):
            mx, vec, wts = [], [], []
            def addmx(items, w=1.0):
                mx.extend(items); wts.extend([w] * len(items))
            if i == NB - 2:
                need("w1"); need("w3"); need("w2")
            if i == 1:
                need("wo"); need("mga"); need("xr")
                addmx(qkv_items(i + 2))
                if not VMODGA:
                    addmx([mod_item(None, 2 * D, D)], 1.5)
                addmx(wo_items(i - 1))
                vec += [(0.1 + 0.5 * cb / NT, functools.partial(wo_prep, cbi)) for cb, cbi in enumerate(range(NT))]
                if VMODGA:
                    vec += mod_vec([2 * D + t * 128 for t in range(NT)], 0.03, 0.65)
            else:
                if i >= 1:
                    addmx(wo_items(i - 1))
                if i + 2 < NB:
                    addmx(qkv_items(i + 2))
            if i == 2:
                need("mb")
            if VMODB:
                if 2 <= i <= 4:
                    vec += mod_vec([(1 + i) * D + t * 128 for t in range(NT)], 0.03, 0.95)
            elif i == MODB_AT:
                addmx([mod_item(None, 3 * D + t * 512, 512) for t in range(6)], 0.5)
            if i < NB:
                vec += att_vec(i, span=(ASPAN if i < NB - 2 else TSPAN))
            if i + 3 < NB:
                vec += ln1_vec(i + 3, LNOFF / 32, LSPAN)
            if i == 5:
                vec += ln2_vec(0, 0.05, 0.4)
            if i == 5:
                vec += ln2_vec(1, 0.5, 0.4)
            if i == NB - 2:
                for f in range(TAILSPLIT):
                    addmx(tail_f[f])
            if i == NB - 1:
                for f in range(TAILSPLIT, F // FC):
                    addmx(tail_f[f])
                addmx([tail_fin], 0.0)
            run_paced(mx, vec, wts)

    def ffn(i, has_next):
        static = isinstance(i, int)
        r0 = i * T if static else pl.multiple_of(i * T, T)
        p0 = i * (T // 2) if static else pl.multiple_of(i * (T // 2), T // 2)
        h = pltpu.bitcast(h2buf[pl.ds(p0, T // 2), :], bf16)
        if has_next:
            nx = i + 1 if static else jnp.minimum(i + 1, NB - 1)
            rn0 = nx * T if static else pl.multiple_of(nx * T, T)
            pn0 = nx * (T // 2) if static else pl.multiple_of(nx * (T // 2), T // 2)
            ln_rows(x1buf, h2buf if PEEL else h2nxt, rn0, pn0 if PEEL else 0, T, 4 * D, 3 * D, None)
        ffn_coarse(i, r0, h)
        if has_next and not PEEL:
            h2buf[pl.ds(pn0, T // 2), :] = h2nxt[...]

    with scope("s4_loop"):
        lax.fori_loop(1, NB - 1 if PEEL else NB, lambda i, c: (ffn(i, True), 0)[1], 0)
    if PEEL:
        with scope("s5_last"):
            ffn(NB - 1, False)
    for i in range(NB):
        pltpu.make_async_copy(outv.at[pl.ds(i * T, T), :], o_hbm.at[pl.ds(i * T, T), :], osems.at[i]).wait()


def pallas_adaLN_cond__sliding_local_dilated__glu_gated_swiglu__prompt_kernel(
        A_x, A_wqkv, A_wo, B_x, B_w1, B_w3, B_w2, c, w_mod):
    NB = S // T
    anyspec = pl.BlockSpec(memory_space=pl.ANY)
    kv_shape = pltpu.VMEM((NT, T + HALO, 128), f32)
    flags = {"XLA_TPU_EVENLY_DISTRIBUTE_CRITICAL_NODES": True} if EVEN else {}
    out = pl.pallas_call(
        _kernel,
        out_shape=jax.ShapeDtypeStruct((S, D), bf16),
        in_specs=[anyspec] * 8,
        out_specs=anyspec,
        scratch_shapes=[
            pltpu.VMEM((S, D), bf16),
            pltpu.VMEM((D, 3 * D), bf16),
            pltpu.VMEM((D // 2, 3 * D), u32),
            pltpu.VMEM((2 * T, D), f32),
            pltpu.VMEM((D, 128), f32),
            pltpu.VMEM((D, D), bf16),
            pltpu.VMEM((D // 2, D), u32),
            pltpu.VMEM((D, F), bf16),
            pltpu.VMEM((D, F), bf16),
            pltpu.VMEM((F, D), bf16),
            pltpu.VMEM((1, D), bf16),
            pltpu.VMEM((D, 6 * D), bf16),
            pltpu.VMEM((8, 6 * D), f32),
            pltpu.VMEM((T // 2, D), u32), pltpu.VMEM((T // 2, D), u32), pltpu.VMEM((T, D), u32),
            kv_shape, kv_shape, kv_shape, kv_shape, kv_shape, kv_shape,
            pltpu.VMEM((NT, T, 128), f32), pltpu.VMEM((NT, T, 128), f32), pltpu.VMEM((NT, T, 128), f32),
            pltpu.VMEM((T, D), bf16), pltpu.VMEM((T, D), bf16),
            pltpu.VMEM((S, D), f32),
            pltpu.VMEM((S // 2, D), u32), pltpu.VMEM((T // 2, D), u32),
            pltpu.VMEM((S, D), bf16),
            pltpu.SemaphoreType.DMA((44,)),
            pltpu.SemaphoreType.DMA((NB,)),
        ],
        compiler_params=pltpu.CompilerParams(vmem_limit_bytes=120 * 1024 * 1024, flags=flags),
    )(A_x.reshape(S, D), A_wqkv, A_wo, B_w1, B_w3, B_w2, c, w_mod)
    return out.reshape(1, S, D)
```

```python
import functools
import math
import jax
import jax.numpy as jnp
import numpy as np
from jax import lax
from jax.experimental import pallas as pl
from jax.experimental.pallas import tpu as pltpu

S, D, F, H, DH, W, DIL = 2048, 1024, 3584, 32, 32, 8, 2
EPS = 1e-5
T = 256
FC = 512
HALO = 16
NT = D // 128
RC = 8
KCH = (128, 128, 256, 256, 256)
NSB = 4
WOFF = (2, 3, 4, 5)
PRG0, PRG = 128, 64
ASPAN = 0.875
TSPAN = 0.9
LSPAN = 0.75
LNP = 8
LN0P = 4
LNOFF = 1
MODB_AT = 2
f32, bf16, u32 = jnp.float32, jnp.bfloat16, jnp.uint32


def _group_allreduce(s):
    lane = lax.broadcasted_iota(jnp.int32, s.shape, 1)
    s = s + jnp.where((lane & 1) == 0, pltpu.roll(s, 127, 1), pltpu.roll(s, 1, 1))
    s = s + jnp.where((lane & 2) == 0, pltpu.roll(s, 126, 1), pltpu.roll(s, 2, 1))
    return s


def _butterfly(X):
    X = list(X)
    lane = lax.broadcasted_iota(jnp.int32, X[0].shape, 1)
    for b, s in ((1, 4), (2, 8), (4, 16)):
        m = (lane & s) == 0
        for i in range(NT):
            if i & b == 0:
                A, B = X[i], X[i | b]
                X[i] = jnp.where(m, A, pltpu.roll(B, s, 1))
                X[i | b] = jnp.where(m, pltpu.roll(A, 128 - s, 1), B)
    return X


def _rowperm(X):
    C = X[0].shape[1]
    U = [pltpu.bitcast(x, u32) for x in X]
    out = [[None] * 8 for _ in range(8)]
    sub = lax.broadcasted_iota(jnp.int32, (8, C), 0)
    m4 = (sub & 4) == 0
    m2 = (sub & 2) == 0
    for a in range(4):
        for j2 in range(2):
            Z = [U[b][(a * 2 + j2) * 8:(a * 2 + j2 + 1) * 8] for b in range(8)]
            for bit, s, m in ((2, 4, m4), (1, 2, m2)):
                for b in range(8):
                    if b & bit == 0:
                        A, B = Z[b], Z[b | bit]
                        Z[b] = jnp.where(m, A, pltpu.roll(B, s, 0))
                        Z[b | bit] = jnp.where(m, pltpu.roll(A, 8 - s, 0), B)
            for b in range(8):
                b2, j1, j0 = b >> 2, (b >> 1) & 1, b & 1
                out[j2 * 4 + j1 * 2 + j0][a * 2 + b2] = Z[b]
    return [jnp.concatenate(o, 0) for o in out]


def _kernel(x_hbm, wqkv_hbm, wo_hbm, w1_hbm, w3_hbm, w2_hbm, c_hbm, wmod_hbm, o_hbm,
            xv, wraw, wp, xh, cb, wo_raw, wo, w1, w3, w2, cv, wmod, mod,
            hA, hB, hS, oA, oB, x1buf, h2buf, h2nxt, outv, sems, osems, *qkv_bufs):
    NB = S // T
    plan = {}

    def add(name, src, dst):
        plan[name] = pltpu.make_async_copy(src, dst, sems.at[len(plan)])

    def cols(ref, a, n):
        return ref.at[:, pl.ds(a, n)]

    def rows(ref, a, n):
        return ref.at[pl.ds(a, n), :]

    kofs = [sum(KCH[:i]) for i in range(len(KCH))]
    assert sum(KCH) == D
    add("c", c_hbm, cv)
    for q, (k0, kn) in enumerate(zip(kofs, KCH)):
        add(f"ms{q}", cols(wmod_hbm, k0, kn), cols(wmod, k0, kn))
        add(f"mc{q}", cols(wmod_hbm, D + k0, kn), cols(wmod, D + k0, kn))
        if q == 0:
            add("x0", rows(x_hbm, 0, T), rows(xv, 0, T))
            for m in range(3):
                add(f"wq0{m}", wqkv_hbm.at[pl.ds(k0, kn), pl.ds(m * D, D)], wraw.at[pl.ds(k0, kn), pl.ds(m * D, D)])
            for b in range(1, NSB):
                add(f"x{b}", rows(x_hbm, b * T, T), rows(xv, b * T, T))
            continue
        add(f"wq{q}", rows(wqkv_hbm, k0, kn), rows(wraw, k0, kn))
    add("xn", rows(x_hbm, NSB * T, 2 * T), rows(xv, NSB * T, 2 * T))
    add("wo", wo_hbm, wo_raw)
    add("mga", cols(wmod_hbm, 2 * D, D), cols(wmod, 2 * D, D))
    add("xr", rows(x_hbm, (NSB + 2) * T, S - (NSB + 2) * T), rows(xv, (NSB + 2) * T, S - (NSB + 2) * T))
    add("mb", cols(wmod_hbm, 3 * D, 3 * D), cols(wmod, 3 * D, 3 * D))
    add("w1", w1_hbm, w1)
    add("w3", w3_hbm, w3)
    add("w2", w2_hbm, w2)
    for d in plan.values():
        d.start()

    def need(name):
        plan[name].wait()

    need("c")
    cc = cv[...].astype(f32)
    sc = jnp.broadcast_to(cc * jax.nn.sigmoid(cc), (8, D)).astype(bf16)
    pred = (pltpu.bitcast(jnp.broadcast_to(cc[:, 0:128], (8, 128)), jnp.int32) | 1) != 0

    def gate(val, y):
        if y is None:
            return val
        return jnp.where(pred, jnp.full((8, 128), val, f32), y)

    def ld16(ref, idx):
        return pltpu.bitcast(ref[idx], bf16)

    def st16(ref, idx, val):
        ref[idx] = pltpu.bitcast(val.astype(bf16), u32)

    for j in range(NT):
        qkv_bufs[NSB + 1][j, 0:HALO, :] = jnp.zeros((HALO, 128), f32)
        qkv_bufs[2 * NSB + 2][j, 0:HALO, :] = jnp.zeros((HALO, 128), f32)

    NS = NSB + 1
    Hs = (hA, hB); Os = (oA, oB)
    Qs, Ks, Vs = qkv_bufs[0:NS], qkv_bufs[NS:2 * NS], qkv_bufs[2 * NS:3 * NS]
    qscale = DH ** -0.5 * math.log2(math.e)

    def ln_rows(src, dst, r_src, r_dst2, rn, c_scale, c_shift, g):
        x = src[pl.ds(r_src, rn), :].astype(f32)
        sm = jnp.sum(x, axis=-1, keepdims=True)
        if g is None:
            m = sm * (1.0 / D)
        else:
            gv = gate(1.0 / D, g)
            m = sm * jnp.concatenate([gv] * (rn // 8), axis=0)[:, 0:1]
        xc = x - m
        v = jnp.mean(xc * xc, axis=-1, keepdims=True)
        hh = xc * lax.rsqrt(v + EPS) * (1.0 + mod[0:1, c_scale:c_scale + D]) + mod[0:1, c_shift:c_shift + D]
        st16(dst, (pl.ds(r_dst2, rn // 2), slice(None)), hh)

    def ln1_piece(i, q, g):
        rn = T // LNP
        ln_rows(xv, Hs[i % 2], i * T + q * rn, q * rn // 2, rn, D, 0, g)

    def ln2_piece(i, q, g):
        rn = T // LNP
        ln_rows(x1buf, h2buf, i * T + q * rn, (i * T + q * rn) // 2, rn, 4 * D, 3 * D, g)

    def xhat(blk):
        rn = T // LN0P
        for p in range(LN0P):
            rs = slice(blk * T + p * rn, blk * T + (p + 1) * rn)
            x0 = xv[rs, :].astype(f32)
            xc = x0 - jnp.mean(x0, axis=-1, keepdims=True)
            xh[rs, :] = xc * lax.rsqrt(jnp.mean(xc * xc, axis=-1, keepdims=True) + EPS)

    modc = {}

    def mod_chunk(q):
        k0, kn = kofs[q], KCH[q]
        sa = jnp.dot(sc, wmod[:, k0:k0 + kn], preferred_element_type=f32)
        ca = jnp.dot(sc, wmod[:, D + k0:D + k0 + kn], preferred_element_type=f32)
        mod[:, k0:k0 + kn] = sa
        mod[:, D + k0:D + k0 + kn] = ca
        modc[q] = (sa[0:1, :], 1.0 + ca[0:1, :])

    def h_chunk(q, blk):
        k0, kn = kofs[q], KCH[q]
        sa, ca1 = modc[q]
        st16(hS, (slice(blk * T // 2, (blk + 1) * T // 2), slice(k0, k0 + kn)), xh[blk * T:(blk + 1) * T, k0:k0 + kn] * ca1 + sa)

    def prep(q, m):
        k0, kn = kofs[q], KCH[q]
        prg = PRG0 if q == 0 else PRG
        for r in range(k0, k0 + kn, prg):
            X = [pltpu.bitcast(wraw[r:r + prg, m * D + j * 128:m * D + (j + 1) * 128], u32) for j in range(NT)]
            X = _butterfly(X)
            for j in range(NT):
                wp[r // 2:(r + prg) // 2, m * D + j * 128:m * D + (j + 1) * 128] = X[j]

    def mm(q, blk, m):
        k0, kn = kofs[q], KCH[q]
        h = ld16(hS, (slice(blk * T // 2, (blk + 1) * T // 2), slice(k0, k0 + kn)))
        bufs, r0 = ((Qs, 0), (Ks, HALO), (Vs, HALO))[m]
        y = jnp.dot(h, ld16(wp, (slice(k0 // 2, (k0 + kn) // 2), slice(m * D, (m + 1) * D))), preferred_element_type=f32)
        dst = bufs[blk]
        for j in range(NT):
            if q == 0:
                dst[j, r0:r0 + T, :] = y[:, j * 128:(j + 1) * 128]
            else:
                dst[j, r0:r0 + T, :] = dst[j, r0:r0 + T, :] + y[:, j * 128:(j + 1) * 128]
        return y[T - 8:T, D - 128:D]

    NQ = len(KCH)
    need("ms0"); need("mc0")
    mod_chunk(0)
    need("x0")
    xhat(0)
    h_chunk(0, 0)
    need("wq00")
    prep(0, 0)
    need("wq01")
    NI = 3 * NSB
    mx = [functools.partial(mm, 0, blk, m) for blk in range(NSB) for m in range(3)]
    mx += [functools.partial(mm, q, blk, m) for q in range(1, NQ) for m in range(3) for blk in range(NSB)]
    after, pre, waits = {}, {}, {}
    def at(pos, fn):
        after.setdefault(pos, []).append(fn)
    pre[0] = lambda: prep(0, 1)
    pre[1] = lambda: prep(0, 2)
    at(0, lambda g: need("wq02"))
    for b in range(1, NSB):
        at(3 * b - 2, lambda g, b=b: need(f"x{b}"))
        at(3 * b - 1, lambda g, b=b: (xhat(b), h_chunk(0, b)))
    for q in range(1, NQ):
        w = NI * q - WOFF[q - 1]
        waits[w - 1] = (q,)
        at(w, lambda g, q=q: mod_chunk(q))
        at(w, lambda g, q=q: [h_chunk(q, b) for b in range(NSB)])
        at(w, lambda g, q=q: prep(q, 0))
        at(max(w + 1, NI * q - 1), lambda g, q=q: prep(q, 1))
        at(NI * q + NSB - 1, lambda g, q=q: prep(q, 2))
    for p in range(LNP):
        at(NI * NQ - NI + ((NI - 1) * p) // LNP, lambda g, p=p: ln1_piece(NSB, p, g))
    at(NI * NQ - NI - 1, lambda g: need("xn"))
    for e, item in enumerate(mx):
        y = item()
        if e in pre:
            pre[e]()
        for fn in after.get(e, []):
            fn(y)
        for q in waits.get(e, ()):
            need(f"ms{q}"); need(f"mc{q}"); need(f"wq{q}")
    for b in range(1, NSB):
        for j in range(NT):
            Ks[b][j, 0:HALO, :] = Ks[b - 1][j, T:T + HALO, :]
            Vs[b][j, 0:HALO, :] = Vs[b - 1][j, T:T + HALO, :]

    def attn_chunk(i, c, g):
        qbuf, k_ref, v_ref, obuf = Qs[i % NS], Ks[i % NS], Vs[i % NS], Os[i % 2]
        rs = slice(c * RC, (c + 1) * RC)
        sg = gate(qscale, g)
        if g is not None and RC > 8:
            sg = jnp.concatenate([sg] * (RC // 8), axis=0)
        qt = [qbuf[j, rs, :] * sg for j in range(NT)]
        ls = []
        for w in range(W):
            o = HALO - DIL * w + c * RC
            s = None
            for j in range(NT):
                p = qt[j] * k_ref[j, o:o + RC, :]
                s = p if s is None else s + p
            s = _group_allreduce(s)
            if i == 0 and c * RC < DIL * w:
                row = c * RC + lax.broadcasted_iota(jnp.int32, (RC, 128), 0)
                s = jnp.where(row >= DIL * w, s, -1e9 * math.log2(math.e))
            ls.append(s)
        m = functools.reduce(jnp.maximum, ls)
        es = [jnp.exp2(l - m) for l in ls]
        r = 1.0 / functools.reduce(jnp.add, es)
        ps = [e * r for e in es]
        for j in range(NT):
            acc = None
            for w in range(W):
                o = HALO - DIL * w + c * RC
                p = ps[w] * v_ref[j, o:o + RC, :]
                acc = p if acc is None else acc + p
            obuf[rs, j * 128:(j + 1) * 128] = acc.astype(bf16)

    def qkv_items(i):
        p, pp = i % NS, (i - 1) % NS
        st = {}
        def mk(n):
            def run():
                if n == 0:
                    for j in range(NT):
                        Ks[p][j, 0:HALO, :] = Ks[pp][j, T:T + HALO, :]
                        Vs[p][j, 0:HALO, :] = Vs[pp][j, T:T + HALO, :]
                    st["h"] = pltpu.bitcast(Hs[i % 2][...], bf16)
                y = jnp.dot(st["h"], ld16(wp, (slice(None), slice(n * 128, (n + 1) * 128))), preferred_element_type=f32)
                dst, r0 = ((Qs[p], 0), (Ks[p], HALO), (Vs[p], HALO))[n // NT]
                dst[n % NT, r0:r0 + T, :] = y
                return y[T - 8:T, :]
            return run
        return [mk(n) for n in range(3 * NT)]

    def wo_items(i):
        st = {}
        def mk(n):
            def run():
                if n == 0:
                    st["o"] = Os[i % 2][...]
                cs = slice(n * 128, (n + 1) * 128)
                a = jnp.dot(st["o"], ld16(wo, (slice(None), cs)), preferred_element_type=f32)
                x1buf[i * T:(i + 1) * T, cs] = xv[i * T:(i + 1) * T, cs].astype(f32) + mod[0:1, 2 * D + n * 128:2 * D + (n + 1) * 128] * a
                return a[T - 8:T, :]
            return run
        return [mk(n) for n in range(NT)]

    def ffn_coarse(i, r0, h):
        acc = None
        for f in range(F // FC):
            fs = slice(f * FC, (f + 1) * FC)
            g = jnp.dot(h, w1[:, fs], preferred_element_type=f32)
            u = jnp.dot(h, w3[:, fs], preferred_element_type=f32)
            a = (g * jax.nn.sigmoid(g) * u).astype(bf16)
            d = jnp.dot(a, w2[fs, :], preferred_element_type=f32)
            acc = d if acc is None else acc + d
        ffn_fin(i, r0, acc)

    def ffn_fin(i, r0, acc):
        outv[pl.ds(r0, T), :] = (x1buf[pl.ds(r0, T), :] + mod[0:1, 5 * D:6 * D] * acc).astype(bf16)
        pltpu.make_async_copy(outv.at[pl.ds(r0, T), :], o_hbm.at[pl.ds(r0, T), :], osems.at[i]).start()

    def ffn_items(i, r0):
        st = {"acc": [None] * NT, "g": {}, "u": {}, "h": None, "a": {}}
        items = []
        nt = FC // 128
        def gu(f, t, which):
            def run():
                if st["h"] is None:
                    st["h"] = pltpu.bitcast(h2buf[r0 // 2:(r0 + T) // 2, :], bf16)
                cs = slice(f * FC + t * 128, f * FC + (t + 1) * 128)
                y = jnp.dot(st["h"], (w1 if which == "g" else w3)[:, cs], preferred_element_type=f32)
                st[which][(f, t)] = y
                if which == "u":
                    g = st["g"].pop((f, t)); u = st["u"].pop((f, t))
                    st["a"][(f, t)] = (g * jax.nn.sigmoid(g) * u).astype(bf16)
                return y[T - 8:T, :]
            return run
        def dn(f, n):
            def run():
                if n == 0:
                    st["af"] = jnp.concatenate([st["a"].pop((f, t)) for t in range(nt)], axis=1)
                d = jnp.dot(st["af"], w2[f * FC:(f + 1) * FC, n * 128:(n + 1) * 128], preferred_element_type=f32)
                st["acc"][n] = d if st["acc"][n] is None else st["acc"][n] + d
                return d[T - 8:T, :]
            return run
        per_f = []
        for f in range(F // FC):
            it = []
            for t in range(nt):
                it += [gu(f, t, "g"), gu(f, t, "u")]
            it += [dn(f, n) for n in range(NT)]
            per_f.append(it)
        def fin():
            ffn_fin(i, r0, jnp.concatenate(st["acc"], axis=1))
            return None
        return per_f, fin

    def run_paced(mx, vec, wts=None):
        wts = wts or [1.0] * len(mx)
        tot = sum(wts)
        vec = sorted(vec, key=lambda t: t[0])
        vi = 0
        cum = 0.0
        for e, item in enumerate(mx):
            y = item()
            cum += wts[e]
            while vi < len(vec) and vec[vi][0] * tot < cum:
                vec[vi][1](y); vi += 1
        while vi < len(vec):
            vec[vi][1](None); vi += 1

    NC = T // RC

    def att_vec(i, lo=0.0, span=None):
        span = ASPAN if span is None else span
        return [(lo + span * c / NC, functools.partial(attn_chunk, i, c)) for c in range(NC)]

    def ln1_vec(i, lo, span):
        return [(lo + span * q / LNP, functools.partial(ln1_piece, i, q)) for q in range(LNP)]

    def ln2_vec(i, lo, span):
        return [(lo + span * q / LNP, functools.partial(ln2_piece, i, q)) for q in range(LNP)]

    def wo_prep(cb, g):
        X = [wo_raw[b * 128:(b + 1) * 128, cb * 128:(cb + 1) * 128] for b in range(NT)]
        Y = _rowperm(X)
        for j in range(NT):
            wo[j * 64:(j + 1) * 64, cb * 128:(cb + 1) * 128] = Y[j]

    def mod_item(c0, cn):
        def run():
            y = jnp.dot(sc, wmod[:, c0:c0 + cn], preferred_element_type=f32)
            mod[:, c0:c0 + cn] = y
            return y[:, 0:128]
        return run

    tail_f, tail_fin = ffn_items(0, 0)
    for i in range(0, NB + 1):
        mx, vec, wts = [], [], []
        def addmx(items, w=1.0):
            mx.extend(items); wts.extend([w] * len(items))
        if i == NB - NSB:
            need("w1"); need("w3"); need("w2")
        if i == 1:
            need("wo"); need("mga"); need("xr")
            addmx(qkv_items(i + NSB))
            addmx([mod_item(2 * D, D)], 1.5)
            addmx(wo_items(i - 1))
            vec += [(0.1 + 0.5 * cb / NT, functools.partial(wo_prep, cbi)) for cb, cbi in enumerate(range(NT))]
        else:
            if i >= 1:
                addmx(wo_items(i - 1))
            if i + NSB < NB:
                addmx(qkv_items(i + NSB))
        if i == MODB_AT:
            need("mb")
            addmx([mod_item(3 * D + t * 512, 512) for t in range(6)], 0.5)
        if i < NB:
            vec += att_vec(i, span=(ASPAN if i < NB - NSB else TSPAN))
        if i + NSB + 1 < NB:
            vec += ln1_vec(i + NSB + 1, LNOFF / 32, LSPAN)
        if i == NB - NSB - 1:
            vec += ln2_vec(0, 0.05, 0.4)
        if i == NB - NSB - 1:
            vec += ln2_vec(1, 0.5, 0.4)
        if NB - NSB <= i < NB:
            nf = F // FC
            t = i - (NB - NSB)
            for f in range((t * nf) // NSB, ((t + 1) * nf) // NSB):
                addmx(tail_f[f])
            if i == NB - 1:
                addmx([tail_fin], 0.0)
        run_paced(mx, vec, wts)

    def ffn(i, carry):
        r0 = pl.multiple_of(i * T, T)
        p0 = pl.multiple_of(i * (T // 2), T // 2)
        h = pltpu.bitcast(h2buf[pl.ds(p0, T // 2), :], bf16)
        nx = jnp.minimum(i + 1, NB - 1)
        ln_rows(x1buf, h2nxt, pl.multiple_of(nx * T, T), 0, T, 4 * D, 3 * D, None)
        ffn_coarse(i, r0, h)
        h2buf[pl.ds(pl.multiple_of(nx * (T // 2), T // 2), T // 2), :] = h2nxt[...]
        return carry

    lax.fori_loop(1, NB, ffn, 0)
    for i in range(NB):
        pltpu.make_async_copy(outv.at[pl.ds(i * T, T), :], o_hbm.at[pl.ds(i * T, T), :], osems.at[i]).wait()


def pallas_adaLN_cond__sliding_local_dilated__glu_gated_swiglu__prompt_kernel(
        A_x, A_wqkv, A_wo, B_x, B_w1, B_w3, B_w2, c, w_mod):
    NB = S // T
    anyspec = pl.BlockSpec(memory_space=pl.ANY)
    kv_shape = pltpu.VMEM((NT, T + HALO, 128), f32)
    flags = {"XLA_TPU_EVENLY_DISTRIBUTE_CRITICAL_NODES": True}
    out = pl.pallas_call(
        _kernel,
        out_shape=jax.ShapeDtypeStruct((S, D), bf16),
        in_specs=[anyspec] * 8,
        out_specs=anyspec,
        scratch_shapes=[
            pltpu.VMEM((S, D), bf16),
            pltpu.VMEM((D, 3 * D), bf16),
            pltpu.VMEM((D // 2, 3 * D), u32),
            pltpu.VMEM((NSB * T, D), f32),
            pltpu.VMEM((D, 128), f32),
            pltpu.VMEM((D, D), bf16),
            pltpu.VMEM((D // 2, D), u32),
            pltpu.VMEM((D, F), bf16),
            pltpu.VMEM((D, F), bf16),
            pltpu.VMEM((F, D), bf16),
            pltpu.VMEM((1, D), bf16),
            pltpu.VMEM((D, 6 * D), bf16),
            pltpu.VMEM((8, 6 * D), f32),
            pltpu.VMEM((T // 2, D), u32), pltpu.VMEM((T // 2, D), u32), pltpu.VMEM((NSB * T // 2, D), u32),
            pltpu.VMEM((T, D), bf16), pltpu.VMEM((T, D), bf16),
            pltpu.VMEM((S, D), f32),
            pltpu.VMEM((S // 2, D), u32), pltpu.VMEM((T // 2, D), u32),
            pltpu.VMEM((S, D), bf16),
            pltpu.SemaphoreType.DMA((44,)),
            pltpu.SemaphoreType.DMA((NB,)),
        ] + [pltpu.VMEM((NT, T, 128), f32)] * (NSB + 1) + [kv_shape] * (2 * NSB + 2),
        compiler_params=pltpu.CompilerParams(vmem_limit_bytes=120 * 1024 * 1024, flags=flags),
    )(A_x.reshape(S, D), A_wqkv, A_wo, B_w1, B_w3, B_w2, c, w_mod)
    return out.reshape(1, S, D)
```
